```python
import os as _os
_os.environ.setdefault('JAX_PLATFORMS', 'cpu')
import jax
import jax.numpy as jnp

def _softmax(x, axis=-1):
    return jax.nn.softmax(x, axis=axis)

def _gelu(x):
    return jax.nn.gelu(x, approximate=True)

def _silu(x):
    return jax.nn.silu(x)

def _sigmoid(x):
    return jax.nn.sigmoid(x)

def _layernorm(x, axis=-1, eps=1e-05):
    m = jnp.mean(x, axis=axis, keepdims=True)
    v = jnp.var(x, axis=axis, keepdims=True)
    return (x - m) / jnp.sqrt(v + eps)

def _scatter_add(tgt, idx, src, axis=0):
    return tgt.at[idx].add(src)

def _segment_sum(src, seg, n):
    return jax.ops.segment_sum(src, seg, n)

class _Rng:

    def __init__(self, key):
        self._k = key

    def _next(self):
        self._k, sub = jax.random.split(self._k)
        return sub

    def normal(self, shape):
        return jax.random.normal(self._next(), shape, dtype=jnp.bfloat16)

    def randint(self, lo, hi, shape):
        return jax.random.randint(self._next(), shape, lo, hi, dtype=jnp.int32)

    def uniform(self, shape, lo=0.0, hi=1.0):
        return jax.random.uniform(self._next(), shape, jnp.bfloat16, lo, hi)

    def permutation(self, n):
        return jax.random.permutation(self._next(), n)
kernel_name = 'adaLN_cond__sliding_block__dense_activation_relu__prompt'

def setup_inputs():
    _rng = _Rng(jax.random.key(int.from_bytes(__import__("os").urandom(4), "little")))
    _w = lambda a: (lambda t: t.astype(jnp.bfloat16) if jnp.issubdtype(t.dtype, jnp.floating) else t)(jnp.asarray(a))

    def _A_setup():
        B, S, D = (1, 2048, 512)
        return {'x': _w((lambda *s: _rng.normal(s) * 0.05)(B, S, D)), 'wqkv': _w((lambda *s: _rng.normal(s) * 0.05)(D, 3 * D)), 'wo': _w((lambda *s: _rng.normal(s) * 0.05)(D, D))}
    _A_in = _A_setup()

    def _B_setup():
        B, S, D, Dff = (1, 2048, 512, 1792)
        return {'x': _w((lambda *s: _rng.normal(s) * 0.05)(B, S, D)), 'w1': _w((lambda *s: _rng.normal(s) * 0.05)(D, Dff)), 'w2': _w((lambda *s: _rng.normal(s) * 0.05)(Dff, D))}
    _B_in = _B_setup()
    return {'A_x': _A_in['x'], 'A_wqkv': _A_in['wqkv'], 'A_wo': _A_in['wo'], 'B_x': _B_in['x'], 'B_w1': _B_in['w1'], 'B_w2': _B_in['w2'], 'c': _w((lambda *s: _rng.normal(s) * 0.05)(1, 512) * 8.0), 'w_mod': _w((lambda *s: _rng.normal(s) * 0.05)(512, 6 * 512) * 512 ** (-0.5) * 8.0)}

def reference(A_x, A_wqkv, A_wo, B_x, B_w1, B_w2, c, w_mod):

    def _A_ref(x, wqkv, wo):
        B, S, D = x.shape
        H = 32
        Dh = D // H
        W = 256
        qkv = (lambda x, *d: x.transpose(*d))((x @ wqkv).reshape(B, S, 3, H, Dh), 2, 0, 3, 1, 4)
        q, k, v = (qkv[0], qkv[1], qkv[2])
        scores = jnp.einsum('bhqd,bhkd->bhqk', q, k) * Dh ** (-0.5)
        idx = jnp.arange(S)
        mask = (idx[:, None] - idx[None, :] >= 0) & (idx[:, None] - idx[None, :] < W)
        scores = jnp.where(mask[None, None], scores, -1000000000.0)
        p = _softmax(scores, axis=-1)
        o = jnp.einsum('bhqk,bhkd->bhqd', p, v)
        return (lambda x, *d: x.transpose(*d))(o, 0, 2, 1, 3).reshape(B, S, D) @ wo

    def _B_ref(x, w1, w2):
        h = jnp.einsum('bsd,df->bsf', x, w1)
        zero = jnp.zeros_like(h)
        h = jnp.maximum(h, zero)
        return jnp.einsum('bsf,fd->bsd', h, w2)
    x = A_x
    mod = (_silu(c) @ w_mod).reshape(c.shape[0], 6, 1, -1)
    sa, ca, ga, sb, cb, gb = (mod[:, 0].copy(), mod[:, 1].copy(), mod[:, 2].copy(), mod[:, 3].copy(), mod[:, 4].copy(), mod[:, 5].copy())
    h = _layernorm(x, axis=-1) * (1 + ca) + sa
    x = x + ga * _A_ref(h, A_wqkv, A_wo)
    h = _layernorm(x, axis=-1) * (1 + cb) + sb
    x = x + gb * _B_ref(h, B_w1, B_w2)
    return x
```

```python
import functools
import jax
import jax.numpy as jnp
from jax import lax
import jax.experimental.pallas as pl
import jax.experimental.pallas.tpu as pltpu

S = 2048
D = 512
H = 32
DH = 16
DFF = 1792
T = 256
QB = 128
HB = QB // 2
NG = 4
NSTEP = S // T
LOG2E = 1.4426950408889634
QSCALE = 0.25 * LOG2E
NEG = -1e30
EPS = 1e-5
PD = 6
NT = (((1,), (1,)), ((), ()))
F32 = jnp.float32
BF16 = jnp.bfloat16
I32 = jnp.int32
FC = 256


def _ln(xf):
    mu = jnp.mean(xf, axis=-1, keepdims=True)
    xc = xf - mu
    var = jnp.mean(xc * xc, axis=-1, keepdims=True)
    return xc * lax.rsqrt(var + EPS)


def _pk(v):
    return pltpu.bitcast(v.astype(BF16), I32)


def _up(v):
    return pltpu.bitcast(v, BF16)


def _kernel(x_ref, xn_ref, c_ref, wmod_hbm, wqkv_hbm, wo_hbm, w1_hbm, w2_hbm, o_ref,
            wmod_v, wqkv_v, wo_v, w1_v, w2_v, wqvt_v, mod_v, h_v, qt_v, ke_v, ko_v, vt_v, ot_v,
            sems):
    i = pl.program_id(0)

    cp_moda = pltpu.make_async_copy(wmod_hbm.at[:, 0:2 * D], wmod_v.at[:, 0:2 * D], sems.at[0])
    cp_modb = pltpu.make_async_copy(wmod_hbm.at[:, 2 * D:6 * D], wmod_v.at[:, 2 * D:6 * D], sems.at[1])
    cp_qkv = pltpu.make_async_copy(wqkv_hbm, wqkv_v, sems.at[2])
    cp_wo = pltpu.make_async_copy(wo_hbm, wo_v, sems.at[3])
    cp_w1 = pltpu.make_async_copy(w1_hbm, w1_v, sems.at[4])
    cp_w2 = pltpu.make_async_copy(w2_hbm, w2_v, sems.at[5])

    def silu_c():
        c = c_ref[...].astype(F32)
        sc = c * jax.nn.sigmoid(c)
        return jnp.broadcast_to(sc, (8, D)).astype(BF16)

    def ln1(ref):
        sa = mod_v[0:1, 0 * D:1 * D]
        ca = mod_v[0:1, 1 * D:2 * D]
        h_v[...] = _pk(_ln(ref[...].astype(F32)) * (1.0 + ca) + sa)

    @pl.when(i == 0)
    def _():
        cp_moda.start()
        cp_qkv.start()
        cp_moda.wait()
        cp_wo.start()
        cp_modb.start()
        cp_w1.start()
        cp_w2.start()
        mod_v[:, 0:2 * D] = jnp.dot(silu_c(), wmod_v[:, 0:2 * D], preferred_element_type=F32)
        ln1(x_ref)
        cp_qkv.wait()
        wqvt_v[0:D // 2, :] = _pk(wqkv_v[:, 0:D].astype(F32).T)
        wqvt_v[D // 2:D, :] = _pk(wqkv_v[:, 2 * D:3 * D].astype(F32).T)

    def step(first):
        nkb = T // QB
        lane = lax.broadcasted_iota(I32, (HB, 128), 1)
        even = ((lane // DH) % 2) == 0
        even32 = ((lax.broadcasted_iota(I32, (HB // 2, 128), 1) // DH) % 2) == 0
        odd32 = ((lax.broadcasted_iota(I32, (HB // 2, 128), 1) // DH) % 2) == 1
        lo_half = lax.broadcasted_iota(I32, (8, QB), 1) < (QB // 2)
        bb = lax.broadcasted_iota(I32, (QB, QB), 0)
        aa = lax.broadcasted_iota(I32, (QB, QB), 1)
        tri = bb > aa
        b6 = lax.broadcasted_iota(I32, (QB // 2, QB), 0)
        a6 = lax.broadcasted_iota(I32, (QB // 2, QB), 1)
        cond_lo = jnp.logical_and(a6 < QB // 2, b6 <= a6)
        cond_hi = jnp.logical_and(a6 >= QB // 2, b6 + QB // 2 > a6)

        h = _up(h_v[...])

        def kproj():
            k = jnp.dot(h, wqkv_v[:, D:2 * D], preferred_element_type=F32)
            row0 = pl.multiple_of(i * (T // 2), T // 2)
            for g in range(NG):
                for j in range(nkb):
                    kb = _pk(k[j * QB:(j + 1) * QB, g * 128:(g + 1) * 128])
                    rows = pl.ds(row0 + j * HB, HB)
                    ke_v[g, rows, :] = jnp.where(even, kb, pltpu.roll(kb, DH, 1))
                    ko_v[g, rows, :] = jnp.where(even, pltpu.roll(kb, 128 - DH, 1), kb)

        def qproj():
            qt = lax.dot_general(_up(wqvt_v[0:D // 2, :]), h, NT, preferred_element_type=F32)
            qt_v[...] = _pk(qt * QSCALE)

        def vproj():
            vt = lax.dot_general(_up(wqvt_v[D // 2:D, :]), h, NT, preferred_element_type=F32)
            for j in range(nkb):
                vt_v[i * nkb + j] = _pk(vt[:, j * QB:(j + 1) * QB])

        lhs_cache = {}

        def lhs(g, par, j, has_first, has_mid):
            key = (g, par, j)
            if key in lhs_cache:
                return lhs_cache[key]
            kv = ke_v if par == 0 else ko_v
            sel = even32 if par == 0 else odd32
            qb = i * nkb + j
            kl = pl.multiple_of(qb * HB, HB)
            if has_first:
                l_lo = kv[g, pl.ds(kl, HB // 2), :]
                l_hi = kv[g, pl.ds(pl.multiple_of(kl + HB // 2, HB // 2), HB // 2), :]
                f_lo = kv[g, pl.ds(pl.multiple_of(kl - 2 * HB, HB // 2), HB // 2), :]
                f_hi = kv[g, pl.ds(pl.multiple_of(kl - 2 * HB + HB // 2, HB // 2), HB // 2), :]
                parts = [jnp.where(sel, f_lo, l_lo), jnp.where(sel, l_lo, f_hi), jnp.where(sel, f_hi, l_hi)]
            else:
                parts = [kv[g, pl.ds(kl, HB), :]]
            if has_mid:
                parts.append(kv[g, pl.ds(pl.multiple_of(kl - HB, HB), HB), :])
            res = _up(jnp.concatenate(parts, axis=0) if len(parts) > 1 else parts[0])
            lhs_cache[key] = res
            return res

        def stage_a(g, hh, j, has_first, has_mid):
            kwin = lhs(g, hh % 2, j, has_first, has_mid)
            r0 = g * 64 + hh * 8
            qh = qt_v[r0:r0 + 8, j * QB:(j + 1) * QB]
            q_lo = jnp.where(lo_half, qh, 0)
            q_hi = jnp.where(lo_half, 0, qh)
            a, b = (q_lo, q_hi) if hh % 2 == 0 else (q_hi, q_lo)
            e0 = hh - hh % 2
            pieces = []
            if e0 > 0:
                pieces.append(jnp.zeros((8 * e0, QB), I32))
            pieces += [a, b]
            if e0 < 6:
                pieces.append(jnp.zeros((8 * (6 - e0), QB), I32))
            w = _up(jnp.concatenate(pieces, axis=0))
            st = jnp.dot(kwin, w, preferred_element_type=F32)
            if has_first:
                hq = QB // 2
                x1, x3, x2 = st[0:hq], st[hq:2 * hq], st[2 * hq:3 * hq]
                sm = jnp.concatenate([jnp.where(cond_lo, x3, x1), jnp.where(cond_hi, x3, x2)], axis=0)
                rest = st[3 * hq:]
            else:
                sm = jnp.where(tri, NEG, st[0:QB])
                rest = st[QB:]
            s = jnp.concatenate([sm, rest], axis=0) if has_mid else sm
            m = jnp.max(s, axis=0, keepdims=True)
            return s, m

        def stage_b(g, hh, j, has_first, has_mid, res):
            qb = i * nkb + j
            s, m = res
            p = jnp.exp2(s - m)
            l = jnp.sum(p, axis=0, keepdims=True)
            r0 = g * 64 + hh * 8
            vts = [vt_v[qb, r0:r0 + 8, :]]
            pm = p[0:QB]
            if has_first:
                ps = [jnp.where(tri, 0.0, pm)]
            else:
                ps = [pm]
            if has_mid:
                vts.append(vt_v[qb - 1, r0:r0 + 8, :])
                ps.append(p[QB:2 * QB])
            if has_first:
                vts.append(vt_v[qb - 2, r0:r0 + 8, :])
                ps.append(jnp.where(tri, pm, 0.0))
            vcat = _up(jnp.concatenate(vts, axis=1) if len(vts) > 1 else vts[0])
            pcat = (jnp.concatenate(ps, axis=0) if len(ps) > 1 else ps[0]).astype(BF16)
            ot = jnp.dot(vcat, pcat, preferred_element_type=F32)
            ot_v[g * 128 + hh * DH:g * 128 + (hh + 1) * DH, j * QB:(j + 1) * QB] = ot * (1.0 / l)

        state = {}

        def wstage(j):
            if first and j == 0:
                cp_wo.wait()
                cp_modb.wait()
                mod_v[:, 2 * D:6 * D] = jnp.dot(silu_c(), wmod_v[:, 2 * D:6 * D], preferred_element_type=F32)
            ga = mod_v[0:1, 2 * D:3 * D]
            sb = mod_v[0:1, 3 * D:4 * D]
            cb = mod_v[0:1, 4 * D:5 * D]
            o = ot_v[:, j * QB:(j + 1) * QB].T.astype(BF16)
            y = jnp.dot(o, wo_v[...], preferred_element_type=F32)
            x1 = x_ref[j * QB:(j + 1) * QB, :].astype(F32) + ga * y
            state['x1', j] = x1
            state['h2', j] = (_ln(x1) * (1.0 + cb) + sb).astype(BF16)
            state['f', j] = []

        def f1(j, c):
            if first and j == 0 and c == 0:
                cp_w1.wait()
            f = jnp.dot(state['h2', j], w1_v[:, c * FC:(c + 1) * FC], preferred_element_type=F32)
            state['f', j].append(jnp.maximum(f, 0.0).astype(BF16))

        def f2(j, n):
            if first and j == 0 and n == 0:
                cp_w2.wait()
            if n == 0:
                state['fc', j] = jnp.concatenate(state['f', j], axis=1)
            gb = mod_v[0:1, 5 * D + n * 128:5 * D + (n + 1) * 128]
            z = jnp.dot(state['fc', j], w2_v[:, n * 128:(n + 1) * 128], preferred_element_type=F32)
            o_ref[j * QB:(j + 1) * QB, n * 128:(n + 1) * 128] = (
                state['x1', j][:, n * 128:(n + 1) * 128] + gb * z).astype(o_ref.dtype)

        flags = [(False, False), (False, True)] if first else [(True, True)] * nkb
        units = [(g, hh, j) + flags[j] for j in range(nkb) for g in range(NG) for hh in range(8)]
        n = len(units)
        nf1 = DFF // FC
        fa = [functools.partial(f1, 0, c) for c in range(nf1)] + [functools.partial(f2, 0, c) for c in range(4)]

        kproj()
        qproj()
        pend = [stage_a(*units[u]) for u in range(PD)]
        vproj()
        for u in range(n):
            if u + PD < n:
                pend.append(stage_a(*units[u + PD]))
            elif fa:
                fa.pop(0)()
            stage_b(*units[u], pend.pop(0))
            if u == n // 2 + 1:
                wstage(0)
        wstage(1)
        for it in fa:
            it()
        f1(1, 0)
        ln1(xn_ref)
        for c in range(1, nf1):
            f1(1, c)
        for c in range(4):
            f2(1, c)

    @pl.when(i == 0)
    def _():
        step(True)

    @pl.when(i > 0)
    def _():
        step(False)


@jax.jit
def pallas_adaLN_cond__sliding_block__dense_activation_relu__prompt_kernel(
        A_x, A_wqkv, A_wo, B_x, B_w1, B_w2, c, w_mod):
    any_spec = pl.BlockSpec(memory_space=pl.ANY)
    return pl.pallas_call(
        _kernel,
        grid=(NSTEP,),
        in_specs=[
            pl.BlockSpec((None, T, D), lambda i: (0, i, 0)),
            pl.BlockSpec((None, T, D), lambda i: (0, jnp.minimum(i + 1, NSTEP - 1), 0)),
            pl.BlockSpec((1, D), lambda i: (0, 0)),
            any_spec, any_spec, any_spec, any_spec, any_spec,
        ],
        out_specs=pl.BlockSpec((None, T, D), lambda i: (0, i, 0)),
        out_shape=jax.ShapeDtypeStruct((1, S, D), BF16),
        scratch_shapes=[
            pltpu.VMEM((D, 6 * D), BF16),
            pltpu.VMEM((D, 3 * D), BF16),
            pltpu.VMEM((D, D), BF16),
            pltpu.VMEM((D, DFF), BF16),
            pltpu.VMEM((DFF, D), BF16),
            pltpu.VMEM((D, D), I32),
            pltpu.VMEM((8, 6 * D), F32),
            pltpu.VMEM((T // 2, D), I32),
            pltpu.VMEM((D // 2, T), I32),
            pltpu.VMEM((NG, S // 2, 128), I32),
            pltpu.VMEM((NG, S // 2, 128), I32),
            pltpu.VMEM((S // QB, D // 2, QB), I32),
            pltpu.VMEM((D, T), F32),
            pltpu.SemaphoreType.DMA((6,)),
        ],
        compiler_params=pltpu.CompilerParams(
            dimension_semantics=("arbitrary",), vmem_limit_bytes=64 * 1024 * 1024),
    )(A_x, A_x, c, w_mod, A_wqkv, A_wo, B_w1, B_w2)
```

```python
import functools
import jax
import jax.numpy as jnp
from jax import lax
import jax.experimental.pallas as pl
import jax.experimental.pallas.tpu as pltpu

S = 2048
D = 512
H = 32
DH = 16
DFF = 1792
T = 256
QB = 128
HB = QB // 2
NG = 4
NBLK = S // T
NKB = T // QB
LOG2E = 1.4426950408889634
QSCALE = 0.25 * LOG2E
NEG = -1e30
EPS = 1e-5
LAG = 44
LEAD = 40
FRAC = 0.85
MAXIN = 8
F2R = 128
ORD = 'acdebfghABCxyD'
ORDN = 'abABCD'
ORDL = 'abABCD'
FRAC0 = 0.85
FRAC1 = 0.85
FRACN = 0.85
TIE = 1
F1R = 256
NT = (((1,), (1,)), ((), ()))
F32 = jnp.float32
BF16 = jnp.bfloat16
I32 = jnp.int32


def _ln(xf, tie=None):
    mu = jnp.mean(xf, axis=-1, keepdims=True)
    if tie is not None:
        mu = jnp.where(tie[0], tie[1], mu)
    xc = xf - mu
    var = jnp.mean(xc * xc, axis=-1, keepdims=True)
    return xc * lax.rsqrt(var + EPS)


def _pk(v):
    return pltpu.bitcast(v.astype(BF16), I32)


def _up(v):
    return pltpu.bitcast(v, BF16)


def _dot(a, b):
    return jnp.dot(a, b, preferred_element_type=F32)


def _dot_nt(a, b):
    return lax.dot_general(a, b, NT, preferred_element_type=F32)


def _kernel(c_ref, x_hbm, wmod_hbm, wqkv_hbm, wo_hbm, w1_hbm, w2_hbm, o_ref,
            x_v, wmod_v, wqkv_v, wo_v, w1_v, w2_v, wqvt_v, mod_v, qt_v, k8_v, vt_v, ao_v, h_v,
            sems):
    i = pl.program_id(0)

    def cp(src, dst, k):
        return pltpu.make_async_copy(src, dst, sems.at[k])

    cp_x0 = cp(x_hbm.at[0, 0:T, :], x_v.at[0:T, :], 0)
    cp_moda = cp(wmod_hbm.at[:, 0:2 * D], wmod_v.at[:, 0:2 * D], 1)
    cp_wk = cp(wqkv_hbm.at[:, D:2 * D], wqkv_v.at[:, D:2 * D], 2)
    cp_x1 = cp(x_hbm.at[0, T:2 * T, :], x_v.at[T:2 * T, :], 3)
    cp_wq = cp(wqkv_hbm.at[:, 0:D], wqkv_v.at[:, 0:D], 4)
    cp_wv = cp(wqkv_hbm.at[:, 2 * D:3 * D], wqkv_v.at[:, 2 * D:3 * D], 5)
    cp_x2 = cp(x_hbm.at[0, 2 * T:4 * T, :], x_v.at[2 * T:4 * T, :], 6)
    cp_modb = cp(wmod_hbm.at[:, 2 * D:6 * D], wmod_v.at[:, 2 * D:6 * D], 7)
    cp_wo = cp(wo_hbm, wo_v, 8)
    cp_w1 = cp(w1_hbm, w1_v, 9)
    cp_w2 = cp(w2_hbm, w2_v, 10)
    cp_xr = cp(x_hbm.at[0, 4 * T:S, :], x_v.at[4 * T:S, :], 11)
    all_cp = [cp_x0, cp_moda, cp_wk, cp_x1, cp_wq, cp_wv, cp_x2, cp_modb, cp_wo, cp_w1, cp_w2, cp_xr]

    def silu_c():
        c = c_ref[...].astype(F32)
        sc = c * jax.nn.sigmoid(c)
        return jnp.broadcast_to(sc, (8, D)).astype(BF16)

    def modmm(lo, hi):
        mod_v[:, lo * D:hi * D] = _dot(silu_c(), wmod_v[:, lo * D:hi * D])

    def mo(v, m):
        return v if isinstance(v, int) else pl.multiple_of(v, m)

    def xhalf(blk, j, c0=0, c1=D):
        return x_v[pl.ds(mo(blk * T + j * QB, QB), QB), c0:c1]

    def step(kind):
        with jax.named_scope('st_' + kind):
            step_(kind)

    def step_(kind):
        first = kind == 'first'
        last = kind == 'last'
        do_attn = not last
        do_dense = not first
        do_proj = kind in ('first', 'gen')
        if kind == 'gen':
            qt_r = qt_v.at[pl.ds(i + 1, 2)]
            k8_r = k8_v.at[:, pl.ds(pl.multiple_of(i * (T // 2), T // 2), 3 * (T // 2)), :]
            vt_r = vt_v.at[pl.ds(i * NKB, 3 * NKB)]
            ao_r = ao_v.at[pl.ds(i - 1, 3)]
            h_r = h_v.at[pl.ds(i + 2, 2)]
            ib_, db, pb = (i + 1, 0, 1, 2), (i - 1, 0, 0, 0), (i + 2, 1, 2, 0)
        else:
            qt_r, k8_r, vt_r, ao_r, h_r = qt_v, k8_v, vt_v, ao_v, h_v
            ib_ = ({'first': 1, 'noproj': NBLK - 1}.get(kind, 0),) * 4
            db = ({'noproj': NBLK - 3}.get(kind, i - 1),) * 4
            pb = (2,) * 4

        loads = [0, 0, 0, 0]
        run = [0, 0, 0, 0]

        def acct(n, cnt=1):
            for _ in range(cnt):
                m = min(range(4), key=lambda k: (loads[k], k))
                loads[m] += max(n, 2)
                run[m] = run[m] + 1 if n <= 2 else 0

        lane = lax.broadcasted_iota(I32, (HB, 128), 1)
        low_of = {w: ((lane // w) % 2) == 0 for w in (64, 32, 16)}
        bb = lax.broadcasted_iota(I32, (QB, QB), 0)
        aa = lax.broadcasted_iota(I32, (QB, QB), 1)
        tri = bb > aa
        diag = (lax.broadcasted_iota(I32, (HB, 128), 0) // 8) == (lax.broadcasted_iota(I32, (HB, 128), 1) // DH)
        use_l = (lax.broadcasted_iota(I32, (HB - 8, 128), 1) // DH) > (lax.broadcasted_iota(I32, (HB - 8, 128), 0) // 8)

        st = {}

        def tie_src(rows):
            v = st.get('last')
            if v is None or not TIE:
                return None
            return v[0:rows, 0:1]

        def ln1(blk, j, xn=None, dep=None):
            sa = mod_v[0:1, 0 * D:1 * D]
            ca = mod_v[0:1, 1 * D:2 * D]
            if xn is None:
                xn = _ln(xhalf(blk[0], j).astype(F32), None if dep is None else (i < 0, dep))
            return (xn * (1.0 + ca) + sa).astype(BF16)

        def hget(tag, j, k):
            if ('h', tag, j) in st:
                return st['h', tag, j][:, k * 128:(k + 1) * 128]
            return h_r[0 if kind == 'gen' else 2, k, j * QB:(j + 1) * QB, :]

        def ln1_next(j, sblk=None):
            blk = jnp.minimum(i + 3, NBLK - 1) if kind == 'gen' else sblk
            h = ln1((blk,), j, dep=tie_src(QB))
            for k in range(4):
                h_r[1 if kind == 'gen' else sblk, k, j * QB:(j + 1) * QB, :] = h[:, k * 128:(k + 1) * 128]

        def acc(key, val):
            st[key] = val if key not in st else val + st[key]
            if val.shape[0] >= QB:
                st['last'] = st[key]
            return st[key]

        def k_tile(tag, blk, j, g, k):
            r = acc(('k', tag, j, g), _dot(hget(tag, j, k),
                                           wqkv_v[k * 128:(k + 1) * 128, D + g * 128:D + (g + 1) * 128]))
            if k == 3:
                kb = _pk(r)
                rows = pl.ds(blk[2] * (T // 2) + j * HB, HB)
                vs = [kb]
                for w in (64, 32, 16):
                    nxt = []
                    for v in vs:
                        rv = pltpu.roll(v, w, 1)
                        nxt += [jnp.where(low_of[w], v, rv), jnp.where(low_of[w], rv, v)]
                    vs = nxt
                for hh in range(8):
                    k8_r[g * 8 + hh, rows, :] = vs[hh]

        def q_tile(tag, blk, j, r, k):
            w = _up(wqvt_v[r * 128:(r + 1) * 128, k * 128:(k + 1) * 128])
            res = acc(('q', tag, r, j), _dot_nt(w, hget(tag, j, k)))
            if k == 3:
                qt_r[blk[1], r * 128:(r + 1) * 128, j * QB:(j + 1) * QB] = _pk(res * QSCALE)

        def v_tile(tag, blk, j, r, k):
            w = _up(wqvt_v[D // 2 + r * 128:D // 2 + (r + 1) * 128, k * 128:(k + 1) * 128])
            res = acc(('v', tag, r, j), _dot_nt(w, hget(tag, j, k)))
            if k == 3:
                vt_r[blk[2] * NKB + j, r * 128:(r + 1) * 128, :] = _pk(res)

        def proj_tasks(tag, blk, j):
            kt = [(functools.partial(k_tile, tag, blk, j, g, k), 8) for g in range(NG) for k in range(4)]
            qt = [(functools.partial(q_tile, tag, blk, j, r, k), 16) for r in range(2) for k in range(4)]
            vt = [(functools.partial(v_tile, tag, blk, j, r, k), 16) for r in range(2) for k in range(4)]
            return kt, qt, vt

        def wo_tile(j, n, k):
            y = acc(('y', j, n), _dot(ao_r[db[3], j * QB:(j + 1) * QB, k * 128:(k + 1) * 128],
                                      wo_v[k * 128:(k + 1) * 128, n * 128:(n + 1) * 128]))
            if k == 3:
                ga = mod_v[0:1, 2 * D + n * 128:2 * D + (n + 1) * 128]
                st['x1', j, n] = xhalf(db[0], j, n * 128, (n + 1) * 128).astype(F32) + ga * y
                if n == 3:
                    sb = mod_v[0:1, 3 * D:4 * D]
                    cb = mod_v[0:1, 4 * D:5 * D]
                    x1 = jnp.concatenate([st['x1', j, q] for q in range(4)], axis=1)
                    st['h2', j] = (_ln(x1) * (1.0 + cb) + sb).astype(BF16)

        def f1_tile(r, c, k):
            if F1R == T:
                if 'h2' not in st:
                    st['h2'] = jnp.concatenate([st['h2', 0], st['h2', 1]], axis=0)
                h2 = st['h2']
            else:
                h2 = st['h2', r]
            f = acc(('f1', r, c), _dot(h2[:, k * 128:(k + 1) * 128],
                                       w1_v[k * 128:(k + 1) * 128, c * 128:(c + 1) * 128]))
            if k == 3:
                f = jnp.maximum(f, 0.0).astype(BF16)
                if F1R == T:
                    st['f', 0, c] = f[0:QB]
                    st['f', 1, c] = f[QB:]
                else:
                    st['f', r, c] = f

        def f2_tile(n, r, c):
            if F2R == T:
                f = jnp.concatenate([st['f', 0, c], st['f', 1, c]], axis=0)
            else:
                f = st['f', r, c]
            z = acc(('z', n, r), _dot(f, w2_v[c * 128:(c + 1) * 128, n * 128:(n + 1) * 128]))
            if c == DFF // 128 - 1:
                gb = mod_v[0:1, 5 * D + n * 128:5 * D + (n + 1) * 128]
                if F2R == T:
                    x1 = jnp.concatenate([st['x1', 0, n], st['x1', 1, n]], axis=0)
                else:
                    x1 = st['x1', r, n]
                o_ref[r * F2R:(r + 1) * F2R, n * 128:(n + 1) * 128] = (x1 + gb * z).astype(o_ref.dtype)

        def wo_tasks(j):
            return [(functools.partial(wo_tile, j, n, k), 8) for n in range(4) for k in range(4)]

        def f1_tasks(r):
            return [(functools.partial(f1_tile, r, c, k), F1R // 16) for c in range(DFF // 128) for k in range(4)]

        def f2_tasks(r):
            return [(functools.partial(f2_tile, n, r, c), F2R // 16)
                    for n in range(4) for c in range(DFF // 128)]

        def lhs(ib, head, j, has_first, has_mid):
            kl = (ib[2] * NKB + j) * HB
            if has_first:
                parts = [k8_r[head, pl.ds(kl, 8), :],
                         jnp.where(use_l, k8_r[head, pl.ds(kl + 8, HB - 8), :], k8_r[head, pl.ds(kl - 2 * HB, HB - 8), :]),
                         k8_r[head, pl.ds(kl - HB - 8, 8), :]]
            else:
                parts = [k8_r[head, pl.ds(kl, HB), :]]
            if has_mid:
                parts.append(k8_r[head, pl.ds(kl - HB, HB), :])
            return _up(jnp.concatenate(parts, axis=0) if len(parts) > 1 else parts[0])

        def qk_rows(has_first, has_mid):
            return (9 if has_first else 8) + (8 if has_mid else 0)

        def stage_a(g, hh, j, has_first, has_mid, ib):
            kwin = lhs(ib, g * 8 + hh, j, has_first, has_mid)
            r0 = g * 64 + hh * 8
            qh = qt_r[ib[1], r0:r0 + 8, j * QB:(j + 1) * QB]
            w = _up(jnp.where(diag, jnp.concatenate([qh] * 8, axis=0), 0))
            s_t = _dot(kwin, w)
            if has_first:
                sm = jnp.where(tri, s_t[DH:QB + DH], s_t[0:QB])
                rest = s_t[QB + DH:]
            else:
                sm = jnp.where(tri, NEG, s_t[0:QB])
                rest = s_t[QB:]
            s = jnp.concatenate([sm, rest], axis=0) if has_mid else sm
            m = jnp.max(s, axis=0, keepdims=True)
            st['s', g, hh, j] = (s, m)

        def pv_tiles(g, hh, j, has_first, has_mid, ib):
            qb = ib[2] * NKB + j
            r0 = g * 64 + hh * 8
            key = ('p', g, hh, j)

            def prep():
                s, m = st.pop(('s', g, hh, j))
                p = jnp.exp2(s - m)
                st[key] = (p, jnp.sum(p, axis=0, keepdims=True))

            def tile(which, is_first, is_last):
                if is_first:
                    prep()
                p, l = st[key]
                pm = p[0:QB]
                if which == 'L':
                    pp = jnp.where(tri, 0.0, pm) if has_first else pm
                    vv = vt_r[qb, r0:r0 + 8, :]
                elif which == 'M':
                    pp = p[QB:2 * QB]
                    vv = vt_r[qb - 1, r0:r0 + 8, :]
                else:
                    pp = jnp.where(tri, pm, 0.0)
                    vv = vt_r[qb - 2, r0:r0 + 8, :]
                ot = acc(('o', ib[2], g, hh, j), _dot(_up(vv), pp.astype(BF16)))
                if is_last:
                    st['on', g, j, hh] = ot * (1.0 / l)
                    if hh == 7:
                        og = jnp.concatenate([st['on', g, j, q] for q in range(8)], axis=0)
                        ao_r[ib[3], j * QB:(j + 1) * QB, g * 128:(g + 1) * 128] = og.T.astype(BF16)

            kinds = ['L'] + (['M'] if has_mid else []) + (['F'] if has_first else [])
            return [functools.partial(tile, w, q == 0, q == len(kinds) - 1) for q, w in enumerate(kinds)]

        def schedule(units, dense, FRAC):
            n = len(units)
            tot = (sum(max(c, 2) for _, c in dense if c)
                   + sum(qk_rows(u[3], u[4]) + 2 * (1 + u[3] + u[4]) for u in units)) / 4.0
            base = min(loads)
            rate = FRAC * tot / max(n, 1)
            nq = 0
            npv = 0
            pvq = []
            qk_time = {}
            nd = 0
            while nq < n or npv < n or dense:
                now = min(loads) - base
                m = min(range(4), key=lambda k: (loads[k], k))
                pv_ok = npv < nq and now >= qk_time[npv] + LAG
                qk_due = nq < n and now >= nq * rate - LEAD and nq - npv < MAXIN
                if pv_ok and run[m] < 2:
                    choice = 'pv'
                elif qk_due:
                    choice = 'qk'
                elif dense:
                    choice = 'd'
                elif nq < n and nq - npv < MAXIN:
                    choice = 'qk'
                else:
                    choice = 'pv'
                if choice == 'pv':
                    if not pvq:
                        pvq = pv_tiles(*units[npv])
                    fn = pvq.pop(0)
                    fn()
                    acct(1)
                    if not pvq:
                        npv += 1
                elif choice == 'qk':
                    qk_time[nq] = now
                    stage_a(*units[nq])
                    acct(qk_rows(units[nq][3], units[nq][4]))
                    nq += 1
                else:
                    fn, c = dense.pop(0)
                    fn()
                    if c:
                        acct(c)
                    nd += 1

        def mk_units(ib, flags):
            return [(g, hh, j) + flags[j] + (ib,) for j in range(NKB) for g in range(NG) for hh in range(8)]

        def ln1_task(tag, blk, j):
            st['h', tag, j] = ln1(blk, j)

        def mod_tasks(lo, hi):
            def t(q):
                mod_v[:, q * 128:(q + 1) * 128] = _dot(silu_c(), wmod_v[:, q * 128:(q + 1) * 128])
            return [(functools.partial(t, q), 8) for q in range(lo * 4, hi * 4)]

        def build(order, groups):
            dense = []
            mix = None
            for ch in order:
                if ch == '(':
                    mix = []
                elif ch == ')':
                    lists = [list(groups[c_]) for c_ in mix]
                    while any(lists):
                        for l_ in lists:
                            dense += l_[:4]
                            del l_[:4]
                    mix = None
                elif mix is not None:
                    mix.append(ch)
                else:
                    dense = dense + groups[ch]
            assert len(dense) == sum(len(v) for v in groups.values())
            return dense

        def proj_groups(groups, tag, blk):
            groups['c'], groups['d'], groups['e'] = proj_tasks(tag, blk, 0)
            groups['f'], groups['g'], groups['h'] = proj_tasks(tag, blk, 1)
            if kind == 'gen':
                groups['x'] = [(functools.partial(ln1_next, 0), 0)]
                groups['y'] = [(functools.partial(ln1_next, 1), 0)]
            else:
                groups['x'] = [(functools.partial(ln1_next, 0, 2), 0)]
                groups['y'] = [(functools.partial(ln1_next, 1, 2), 0)]
                groups['z'] = [(functools.partial(ln1_next, 0, 3), 0), (functools.partial(ln1_next, 1, 3), 0)]

        if first:
            for c_ in all_cp:
                c_.start()
            cp_x0.wait()
            xn0 = [_ln(x_v[j * QB:(j + 1) * QB, :].astype(F32)) for j in range(NKB)]
            cp_moda.wait()
            modmm(0, 2)
            for j in range(NKB):
                st['h', 'a', j] = ln1((0,) * 4, j, xn0[j])
            pa = [proj_tasks('a', (0,) * 4, j) for j in range(NKB)]
            pb_ = [proj_tasks('b', (1,) * 4, j) for j in range(NKB)]
            cp_wk.wait()
            for j in range(NKB):
                for fn, c in pa[j][0]:
                    fn()
            cp_x1.wait()
            for j in range(NKB):
                ln1_task('b', (1,) * 4, j)
                for fn, c in pb_[j][0]:
                    fn()
            cp_wq.wait()
            cp_wv.wait()
            wqvt_v[0:D // 2, :] = _pk(wqkv_v[:, 0:D].astype(F32).T)
            wqvt_v[D // 2:D, :] = _pk(wqkv_v[:, 2 * D:3 * D].astype(F32).T)
            for j in range(NKB):
                for q in (1, 2):
                    for fn, c in pa[j][q]:
                        fn()
                        acct(c)
            dense = []
            for j in range(NKB):
                dense += pb_[j][1] + pb_[j][2]
            schedule(mk_units((0,) * 4, [(False, False), (False, True)]), dense, FRAC0)
            cp_x2.wait()
            cp_modb.wait()
            groups = {ch: [] for ch in 'cdefghxymz'}
            proj_groups(groups, 'c', (2,) * 4)
            groups['m'] = mod_tasks(2, 6)
            schedule(mk_units((1,) * 4, [(True, True)] * NKB), build('xycdemfghz', groups), FRAC1)
            cp_wo.wait()
            cp_w1.wait()
            cp_w2.wait()
            cp_xr.wait()
        else:
            groups = {ch: [] for ch in 'abcdefghABCDxy'}
            groups['a'] = wo_tasks(0)
            groups['b'] = wo_tasks(1)
            groups['A'] = f1_tasks(0)
            groups['C'] = f2_tasks(0)
            if F1R != T:
                groups['B'] = f1_tasks(1)
            if F2R != T:
                groups['D'] = f2_tasks(1)
            if do_proj:
                proj_groups(groups, 'b', pb)
            units = mk_units(ib_, [(True, True)] * NKB) if do_attn else []
            schedule(units, build({'gen': ORD, 'noproj': ORDN, 'last': ORDL}[kind].replace('x', 'x' if do_proj else ''), groups),
                     FRAC if kind == 'gen' else FRACN)

    variants = [
        (jnp.logical_and(i > 0, i < NBLK - 2), 'gen'),
        (i == 0, 'first'),
        (i == NBLK - 2, 'noproj'),
        (i > NBLK - 2, 'last'),
    ]
    for cond, kind in variants:
        pl.when(cond)(functools.partial(step, kind))


@jax.jit
def pallas_adaLN_cond__sliding_block__dense_activation_relu__prompt_kernel(A_x, A_wqkv, A_wo, B_x, B_w1, B_w2, c, w_mod):
    any_spec = pl.BlockSpec(memory_space=pl.ANY)
    return pl.pallas_call(
        _kernel,
        grid=(NBLK + 1,),
        in_specs=[
            pl.BlockSpec((1, D), lambda i: (0, 0)),
            any_spec, any_spec, any_spec, any_spec, any_spec, any_spec,
        ],
        out_specs=pl.BlockSpec((None, T, D), lambda i: (0, jnp.maximum(i - 1, 0), 0)),
        out_shape=jax.ShapeDtypeStruct((1, S, D), BF16),
        scratch_shapes=[
            pltpu.VMEM((S, D), BF16),
            pltpu.VMEM((D, 6 * D), BF16),
            pltpu.VMEM((D, 3 * D), BF16),
            pltpu.VMEM((D, D), BF16),
            pltpu.VMEM((D, DFF), BF16),
            pltpu.VMEM((DFF, D), BF16),
            pltpu.VMEM((D, D), I32),
            pltpu.VMEM((8, 6 * D), F32),
            pltpu.VMEM((NBLK, D // 2, T), I32),
            pltpu.VMEM((H, S // 2, 128), I32),
            pltpu.VMEM((S // QB, D // 2, QB), I32),
            pltpu.VMEM((NBLK, T, D), BF16),
            pltpu.VMEM((NBLK + 1, 4, T, 128), BF16),
            pltpu.SemaphoreType.DMA((12,)),
        ],
        compiler_params=pltpu.CompilerParams(
            dimension_semantics=("arbitrary",), vmem_limit_bytes=100 * 1024 * 1024),
    )(c, A_x, w_mod, A_wqkv, A_wo, B_w1, B_w2)
```

```python
import functools
import jax
import jax.numpy as jnp
from jax import lax
import jax.experimental.pallas as pl
import jax.experimental.pallas.tpu as pltpu

S = 2048
D = 512
H = 32
DH = 16
DFF = 1792
T = 256
QB = 128
HB = QB // 2
NG = 4
NBLK = S // T
NKB = T // QB
LOG2E = 1.4426950408889634
QSCALE = 0.25 * LOG2E
NEG = -1e30
EPS = 1e-5
PG = [0.85, 40.0, 44.0, 8.0]
P0 = [0.85, 40.0, 44.0, 8.0]
P1 = [0.85, 40.0, 44.0, 8.0]
PN = [0.7, 40.0, 44.0, 8.0]
ORD = 'acdebfghABCD'
ORD1 = 'mcdefghab'
ORDN = 'abABCD'
L1R = [0.1, 0.9]
L2R = [0.95]
LR = 32
TIE = 1
F1R = 256
F2R = 128
NT = (((1,), (1,)), ((), ()))
F32 = jnp.float32
BF16 = jnp.bfloat16
I32 = jnp.int32


def _ln(xf, tie=None):
    mu = jnp.mean(xf, axis=-1, keepdims=True)
    if tie is not None:
        mu = jnp.where(tie[0], tie[1], mu)
    xc = xf - mu
    var = jnp.mean(xc * xc, axis=-1, keepdims=True)
    return xc * lax.rsqrt(var + EPS)


def _pk(v):
    return pltpu.bitcast(v.astype(BF16), I32)


def _up(v):
    return pltpu.bitcast(v, BF16)


def _dot(a, b):
    return jnp.dot(a, b, preferred_element_type=F32)


def _dot_nt(a, b):
    return lax.dot_general(a, b, NT, preferred_element_type=F32)


def _kernel(c_ref, x_hbm, wmod_hbm, wqkv_hbm, wo_hbm, w1_hbm, w2_hbm, o_ref,
            x_v, wmod_v, wqkv_v, wo_v, w1_v, w2_v, wqvt_v, mod_v, qt_v, k8_v, vt_v, ao_v, h_v, x1_v, h2_v,
            sems):
    i = pl.program_id(0)

    def cp(src, dst, k):
        return pltpu.make_async_copy(src, dst, sems.at[k])

    cp_x0 = cp(x_hbm.at[0, 0:T, :], x_v.at[0:T, :], 0)
    cp_moda = cp(wmod_hbm.at[:, 0:2 * D], wmod_v.at[:, 0:2 * D], 1)
    cp_x1 = cp(x_hbm.at[0, T:2 * T, :], x_v.at[T:2 * T, :], 2)
    cp_wk = cp(wqkv_hbm.at[:, D:2 * D], wqkv_v.at[:, D:2 * D], 3)
    cp_wq = cp(wqkv_hbm.at[:, 0:D], wqkv_v.at[:, 0:D], 4)
    cp_wv = cp(wqkv_hbm.at[:, 2 * D:3 * D], wqkv_v.at[:, 2 * D:3 * D], 5)
    cp_x2 = cp(x_hbm.at[0, 2 * T:4 * T, :], x_v.at[2 * T:4 * T, :], 6)
    cp_modb = cp(wmod_hbm.at[:, 2 * D:6 * D], wmod_v.at[:, 2 * D:6 * D], 7)
    cp_wo = cp(wo_hbm, wo_v, 8)
    cp_w1 = cp(w1_hbm, w1_v, 9)
    cp_w2 = cp(w2_hbm, w2_v, 10)
    cp_xr = cp(x_hbm.at[0, 4 * T:S, :], x_v.at[4 * T:S, :], 11)
    all_cp = [cp_x0, cp_moda, cp_x1, cp_wk, cp_wq, cp_wv, cp_x2, cp_modb, cp_wo, cp_w1, cp_w2, cp_xr]

    def silu_c():
        c = c_ref[...].astype(F32)
        sc = c * jax.nn.sigmoid(c)
        return jnp.broadcast_to(sc, (8, D)).astype(BF16)

    def modmm(lo, hi):
        mod_v[:, lo * D:hi * D] = _dot(silu_c(), wmod_v[:, lo * D:hi * D])

    def xrows(blk, r0, n, c0=0, c1=D):
        start = blk * T + r0
        if not isinstance(start, int):
            start = pl.multiple_of(start, n)
        return x_v[pl.ds(start, n), c0:c1]

    def step(kind):
        with jax.named_scope('st_' + kind):
            step_(kind)

    def step_(kind):
        first = kind == 'first'
        gen = kind == 'gen'
        if gen:
            qt_r = qt_v.at[pl.ds(i + 1, 2)]
            k8_r = k8_v.at[:, pl.ds(pl.multiple_of(i * (T // 2), T // 2), 3 * (T // 2)), :]
            vt_r = vt_v.at[pl.ds(i * NKB, 3 * NKB)]
            ao_r = ao_v.at[pl.ds(i, 2)]
            h_r = h_v.at[pl.ds(i + 2, 2)]
            x1_r = x1_v.at[pl.ds(i - 1, 2)]
            h2_r = h2_v.at[pl.ds(i - 1, 2)]
        else:
            qt_r, k8_r, vt_r, ao_r, h_r, x1_r, h2_r = qt_v, k8_v, vt_v, ao_v, h_v, x1_v, h2_v

        loads = [0, 0, 0, 0]
        run = [0, 0, 0, 0]

        def acct(n):
            m = min(range(4), key=lambda k: (loads[k], k))
            loads[m] += max(n, 2)
            run[m] = run[m] + 1 if n <= 2 else 0

        lane = lax.broadcasted_iota(I32, (HB, 128), 1)
        low_of = {w: ((lane // w) % 2) == 0 for w in (64, 32, 16)}
        bb = lax.broadcasted_iota(I32, (QB, QB), 0)
        aa = lax.broadcasted_iota(I32, (QB, QB), 1)
        tri = bb > aa
        diag = (lax.broadcasted_iota(I32, (HB, 128), 0) // 8) == (lax.broadcasted_iota(I32, (HB, 128), 1) // DH)
        use_l = (lax.broadcasted_iota(I32, (HB - 8, 128), 1) // DH) > (lax.broadcasted_iota(I32, (HB - 8, 128), 0) // 8)

        st = {}

        def acc(key, val):
            st[key] = val if key not in st else val + st[key]
            if val.shape[0] >= QB:
                st['last'] = st[key]
            return st[key]

        def tie(rows):
            v = st.get('last')
            if v is None or not TIE:
                return None
            return (i < 0, v[0:rows, 0:1])

        def ln1_chunk(xblk, hidx, r0, xn=None):
            if xn is None:
                xn = _ln(xrows(xblk, r0, LR).astype(F32), tie(LR))
            h = (xn * (1.0 + mod_v[0:1, D:2 * D]) + mod_v[0:1, 0:D]).astype(BF16)
            for k in range(4):
                h_r[hidx, k, r0:r0 + xn.shape[0], :] = h[:, k * 128:(k + 1) * 128]

        def ln2_chunk(widx, r0):
            xn = _ln(x1_r[widx, r0:r0 + LR, :], tie(LR))
            h = (xn * (1.0 + mod_v[0:1, 4 * D:5 * D]) + mod_v[0:1, 3 * D:4 * D]).astype(BF16)
            for k in range(4):
                h2_r[widx, k, r0:r0 + LR, :] = h[:, k * 128:(k + 1) * 128]

        def ln1_tasks(xblk, hidx, j=None):
            rows = range(0, T, LR) if j is None else range(j * QB, (j + 1) * QB, LR)
            return [(functools.partial(ln1_chunk, xblk, hidx, r0), 0, 0) for r0 in rows]

        def ln2_tasks(widx, j, need=0):
            return [(functools.partial(ln2_chunk, widx, r0), 0, need) for r0 in range(j * QB, (j + 1) * QB, LR)]

        def k_tile(blk, j, g, k):
            r = acc(('k', blk, j, g), _dot(h_r[blk[0], k, j * QB:(j + 1) * QB, :],
                                           wqkv_v[k * 128:(k + 1) * 128, D + g * 128:D + (g + 1) * 128]))
            if k == 3:
                kb = _pk(r)
                rows = pl.ds(blk[2] * (T // 2) + j * HB, HB)
                vs = [kb]
                for w in (64, 32, 16):
                    nxt = []
                    for v in vs:
                        rv = pltpu.roll(v, w, 1)
                        nxt += [jnp.where(low_of[w], v, rv), jnp.where(low_of[w], rv, v)]
                    vs = nxt
                for hh in range(8):
                    k8_r[g * 8 + hh, rows, :] = vs[hh]

        def q_tile(blk, j, r, k):
            w = _up(wqvt_v[r * 128:(r + 1) * 128, k * 128:(k + 1) * 128])
            res = acc(('q', blk, r, j), _dot_nt(w, h_r[blk[0], k, j * QB:(j + 1) * QB, :]))
            if k == 3:
                qt_r[blk[1], r * 128:(r + 1) * 128, j * QB:(j + 1) * QB] = _pk(res * QSCALE)

        def v_tile(blk, j, r, k):
            w = _up(wqvt_v[D // 2 + r * 128:D // 2 + (r + 1) * 128, k * 128:(k + 1) * 128])
            res = acc(('v', blk, r, j), _dot_nt(w, h_r[blk[0], k, j * QB:(j + 1) * QB, :]))
            if k == 3:
                vt_r[blk[2] * NKB + j, r * 128:(r + 1) * 128, :] = _pk(res)

        def proj_tasks(blk, j):
            kt = [(functools.partial(k_tile, blk, j, g, k), 8, 0) for g in range(NG) for k in range(4)]
            qt = [(functools.partial(q_tile, blk, j, r, k), 16, 0) for r in range(2) for k in range(4)]
            vt = [(functools.partial(v_tile, blk, j, r, k), 16, 0) for r in range(2) for k in range(4)]
            return kt, qt, vt

        def wo_tile(blk, j, n, k):
            y = acc(('y', blk[1], j, n), _dot(ao_r[blk[1], j * QB:(j + 1) * QB, k * 128:(k + 1) * 128],
                                              wo_v[k * 128:(k + 1) * 128, n * 128:(n + 1) * 128]))
            if k == 3:
                ga = mod_v[0:1, 2 * D + n * 128:2 * D + (n + 1) * 128]
                x1_r[blk[2], j * QB:(j + 1) * QB, n * 128:(n + 1) * 128] = (
                    xrows(blk[0], j * QB, QB, n * 128, (n + 1) * 128).astype(F32) + ga * y)

        def wo_tasks(blk, j, need=0):
            return [(functools.partial(wo_tile, blk, j, n, k), 8, need) for n in range(4) for k in range(4)]

        def f1_tile(widx, r, c, k):
            f = acc(('f1', r, c), _dot(h2_r[widx, k, r * F1R:(r + 1) * F1R, :],
                                       w1_v[k * 128:(k + 1) * 128, c * 128:(c + 1) * 128]))
            if k == 3:
                f = jnp.maximum(f, 0.0).astype(BF16)
                if F1R == T:
                    st['f', 0, c] = f[0:QB]
                    st['f', 1, c] = f[QB:]
                else:
                    st['f', r, c] = f

        def f2_tile(widx, n, r, c):
            if F2R == T:
                f = jnp.concatenate([st['f', 0, c], st['f', 1, c]], axis=0)
            else:
                f = st['f', r, c]
            z = acc(('z', n, r), _dot(f, w2_v[c * 128:(c + 1) * 128, n * 128:(n + 1) * 128]))
            if c == DFF // 128 - 1:
                gb = mod_v[0:1, 5 * D + n * 128:5 * D + (n + 1) * 128]
                x1 = x1_r[widx, r * F2R:(r + 1) * F2R, n * 128:(n + 1) * 128]
                o_ref[r * F2R:(r + 1) * F2R, n * 128:(n + 1) * 128] = (x1 + gb * z).astype(o_ref.dtype)

        def f1_tasks(widx, r):
            return [(functools.partial(f1_tile, widx, r, c, k), F1R // 16, 0)
                    for c in range(DFF // 128) for k in range(4)]

        def f2_tasks(widx, r):
            return [(functools.partial(f2_tile, widx, n, r, c), F2R // 16, 0)
                    for n in range(4) for c in range(DFF // 128)]

        def ffn_groups(groups, widx):
            groups['A'] = f1_tasks(widx, 0)
            groups['B'] = f1_tasks(widx, 1) if F1R != T else []
            groups['C'] = f2_tasks(widx, 0)
            groups['D'] = f2_tasks(widx, 1) if F2R != T else []

        def lhs(ib, head, j, has_first, has_mid):
            kl = (ib[1] * NKB + j) * HB
            if has_first:
                parts = [k8_r[head, pl.ds(kl, 8), :],
                         jnp.where(use_l, k8_r[head, pl.ds(kl + 8, HB - 8), :], k8_r[head, pl.ds(kl - 2 * HB, HB - 8), :]),
                         k8_r[head, pl.ds(kl - HB - 8, 8), :]]
            else:
                parts = [k8_r[head, pl.ds(kl, HB), :]]
            if has_mid:
                parts.append(k8_r[head, pl.ds(kl - HB, HB), :])
            return _up(jnp.concatenate(parts, axis=0) if len(parts) > 1 else parts[0])

        def qk_rows(has_first, has_mid):
            return (9 if has_first else 8) + (8 if has_mid else 0)

        def stage_a(g, hh, j, has_first, has_mid, ib):
            kwin = lhs(ib, g * 8 + hh, j, has_first, has_mid)
            r0 = g * 64 + hh * 8
            qh = qt_r[ib[0], r0:r0 + 8, j * QB:(j + 1) * QB]
            w = _up(jnp.where(diag, jnp.concatenate([qh] * 8, axis=0), 0))
            s_t = _dot(kwin, w)
            if has_first:
                sm = jnp.where(tri, s_t[DH:QB + DH], s_t[0:QB])
                rest = s_t[QB + DH:]
            else:
                sm = jnp.where(tri, NEG, s_t[0:QB])
                rest = s_t[QB:]
            s = jnp.concatenate([sm, rest], axis=0) if has_mid else sm
            m = jnp.max(s, axis=0, keepdims=True)
            st['s', g, hh, j] = (s, m)

        def pv_tiles(g, hh, j, has_first, has_mid, ib):
            qb = ib[1] * NKB + j
            r0 = g * 64 + hh * 8
            key = ('p', g, hh, j)

            def prep():
                s, m = st.pop(('s', g, hh, j))
                p = jnp.exp2(s - m)
                st[key] = (p, jnp.sum(p, axis=0, keepdims=True))

            def tile(which, is_first, is_last):
                if is_first:
                    prep()
                p, l = st[key]
                pm = p[0:QB]
                if which == 'L':
                    pp = jnp.where(tri, 0.0, pm) if has_first else pm
                    vv = vt_r[qb, r0:r0 + 8, :]
                elif which == 'M':
                    pp = p[QB:2 * QB]
                    vv = vt_r[qb - 1, r0:r0 + 8, :]
                else:
                    pp = jnp.where(tri, pm, 0.0)
                    vv = vt_r[qb - 2, r0:r0 + 8, :]
                ot = acc(('o', ib[1], g, hh, j), _dot(_up(vv), pp.astype(BF16)))
                if is_last:
                    st['on', g, j, hh] = ot * (1.0 / l)
                    if hh == 7:
                        og = jnp.concatenate([st['on', g, j, q] for q in range(8)], axis=0)
                        ao_r[ib[2], j * QB:(j + 1) * QB, g * 128:(g + 1) * 128] = og.T.astype(BF16)

            kinds = ['L'] + (['M'] if has_mid else []) + (['F'] if has_first else [])
            return [functools.partial(tile, w, q == 0, q == len(kinds) - 1) for q, w in enumerate(kinds)]

        def schedule(units, dense, params, gated=()):
            frac, lead, lag, maxin = params
            gated = list(gated)
            n = len(units)
            tot = (sum(max(c, 2) for _, c, _ in dense + gated if c)
                   + sum(qk_rows(u[3], u[4]) + 2 * (1 + u[3] + u[4]) for u in units)) / 4.0
            base = min(loads)
            rate = frac * tot / max(n, 1)
            nq = 0
            npv = 0
            pvq = []
            qk_time = {}
            while nq < n or npv < n or dense or gated:
                now = min(loads) - base
                m = min(range(4), key=lambda k: (loads[k], k))
                pv_ok = npv < nq and now >= qk_time[npv] + lag
                qk_due = nq < n and now >= nq * rate - lead and nq - npv < maxin
                if gated and npv >= gated[0][2]:
                    choice = 'g'
                elif pv_ok and run[m] < 2:
                    choice = 'pv'
                elif qk_due:
                    choice = 'qk'
                elif dense:
                    choice = 'd'
                elif nq < n and nq - npv < maxin:
                    choice = 'qk'
                else:
                    choice = 'pv'
                if choice == 'pv':
                    if not pvq:
                        pvq = pv_tiles(*units[npv])
                    fn = pvq.pop(0)
                    fn()
                    acct(1)
                    if not pvq:
                        npv += 1
                elif choice == 'qk':
                    qk_time[nq] = now
                    stage_a(*units[nq])
                    acct(qk_rows(units[nq][3], units[nq][4]))
                    nq += 1
                else:
                    fn, c, _ = (dense if choice == 'd' else gated).pop(0)
                    fn()
                    if c:
                        acct(c)

        def mk_units(ib, flags):
            return [(g, hh, j) + flags[j] + (ib,) for j in range(NKB) for g in range(NG) for hh in range(8)]

        def mod_tasks(lo, hi):
            def t(q):
                mod_v[:, q * 128:(q + 1) * 128] = _dot(silu_c(), wmod_v[:, q * 128:(q + 1) * 128])
            return [(functools.partial(t, q), 8, 0) for q in range(lo * 4, hi * 4)]

        def build(order, groups):
            dense = []
            ends = {}
            for ch in order:
                dense = dense + groups[ch]
                ends[ch] = len(dense)
            return dense, ends

        def sprinkle(dense, extras):
            ins = []
            for tasks, lo, hi in extras:
                hi = max(hi, lo)
                for q, t in enumerate(tasks):
                    ins.append((lo + (hi - lo) * (q + 0.5) / len(tasks), t))
            ins.sort(key=lambda e: e[0])
            out = []
            for pos, t in enumerate(dense):
                while ins and ins[0][0] <= pos:
                    out.append(ins.pop(0)[1])
                out.append(t)
            return out + [e[1] for e in ins]

        def proj_groups(groups, blk):
            groups['c'], groups['d'], groups['e'] = proj_tasks(blk, 0)
            groups['f'], groups['g'], groups['h'] = proj_tasks(blk, 1)

        full = [(True, True)] * NKB
        if first:
            for c_ in all_cp:
                c_.start()
            cp_x0.wait()
            xn0 = [_ln(x_v[j * QB:(j + 1) * QB, :].astype(F32)) for j in range(NKB)]
            cp_moda.wait()
            modmm(0, 2)
            for j in range(NKB):
                ln1_chunk(0, 0, j * QB, xn0[j])
            cp_x1.wait()
            for fn, _, _ in ln1_tasks(1, 1):
                fn()
            pa = [proj_tasks((0, 0, 0), j) for j in range(NKB)]
            pb = [proj_tasks((1, 1, 1), j) for j in range(NKB)]
            cp_wk.wait()
            for pr in (pa, pb):
                for j in range(NKB):
                    for fn, c, _ in pr[j][0]:
                        fn()
            cp_wq.wait()
            cp_wv.wait()
            wqvt_v[0:D // 2, :] = _pk(wqkv_v[:, 0:D].astype(F32).T)
            wqvt_v[D // 2:D, :] = _pk(wqkv_v[:, 2 * D:3 * D].astype(F32).T)
            for j in range(NKB):
                for q in (1, 2):
                    for fn, c, _ in pa[j][q]:
                        fn()
                        acct(c)
            dense = []
            for j in range(NKB):
                dense += pb[j][1] + pb[j][2]
            schedule(mk_units((0, 0, 0), [(False, False), (False, True)]), dense, P0)
            cp_x2.wait()
            cp_modb.wait()
            cp_wo.wait()
            groups = {'m': mod_tasks(2, 6), 'a': wo_tasks((0, 0, 0), 0), 'b': wo_tasks((0, 0, 0), 1)}
            proj_groups(groups, (2, 2, 2))
            for j in range(NKB):
                for fn, _, _ in ln1_tasks(2, 2, j):
                    fn()
            dense, ends = build(ORD1, groups)
            n = len(dense)
            dense = sprinkle(dense, [(ln1_tasks(3, 3), L1R[0] * n, L1R[1] * n),
                                     (ln2_tasks(0, 0), ends['a'], n), (ln2_tasks(0, 1), ends['b'], n)])
            schedule(mk_units((1, 1, 1), full), dense, P1)
            cp_w1.wait()
            cp_w2.wait()
            cp_xr.wait()
        elif gen:
            groups = {'a': wo_tasks((i, 0, 1), 0), 'b': wo_tasks((i, 0, 1), 1)}
            ffn_groups(groups, 0)
            proj_groups(groups, (0, 1, 2))
            dense, ends = build(ORD, groups)
            n = len(dense)
            dense = sprinkle(dense, [(ln1_tasks(jnp.minimum(i + 3, NBLK - 1), 1), L1R[0] * n, L1R[1] * n),
                                     (ln2_tasks(1, 0), ends['a'], L2R[0] * n), (ln2_tasks(1, 1), ends['b'], L2R[0] * n)])
            schedule(mk_units((0, 1, 1), full), dense, PG)
        elif kind == 'noproj':
            lb = NBLK - 1
            groups = {'a': wo_tasks((lb - 1,) * 3, 0), 'b': wo_tasks((lb - 1,) * 3, 1)}
            ffn_groups(groups, lb - 2)
            dense, ends = build(ORDN, groups)
            n = len(dense)
            dense = sprinkle(dense, [(ln2_tasks(lb - 1, 0), ends['a'], L2R[0] * n),
                                     (ln2_tasks(lb - 1, 1), ends['b'], L2R[0] * n)])
            gated = []
            for j in range(NKB):
                need = (j + 1) * NG * 8
                gated += wo_tasks((lb,) * 3, j, need) + ln2_tasks(lb, j, need)
            schedule(mk_units((lb,) * 3, full), dense, PN, gated)
        else:
            groups = {}
            ffn_groups(groups, i - 1)
            schedule([], build('ABCD', groups)[0], PG)

    variants = [
        (jnp.logical_and(i > 0, i < NBLK - 2), 'gen'),
        (i == 0, 'first'),
        (i == NBLK - 2, 'noproj'),
        (i > NBLK - 2, 'last'),
    ]
    for cond, kind in variants:
        pl.when(cond)(functools.partial(step, kind))


@jax.jit
def pallas_adaLN_cond__sliding_block__dense_activation_relu__prompt_kernel(A_x, A_wqkv, A_wo, B_x, B_w1, B_w2, c, w_mod):
    any_spec = pl.BlockSpec(memory_space=pl.ANY)
    return pl.pallas_call(
        _kernel,
        grid=(NBLK + 1,),
        in_specs=[
            pl.BlockSpec((1, D), lambda i: (0, 0)),
            any_spec, any_spec, any_spec, any_spec, any_spec, any_spec,
        ],
        out_specs=pl.BlockSpec((None, T, D), lambda i: (0, jnp.maximum(i - 1, 0), 0)),
        out_shape=jax.ShapeDtypeStruct((1, S, D), BF16),
        scratch_shapes=[
            pltpu.VMEM((S, D), BF16),
            pltpu.VMEM((D, 6 * D), BF16),
            pltpu.VMEM((D, 3 * D), BF16),
            pltpu.VMEM((D, D), BF16),
            pltpu.VMEM((D, DFF), BF16),
            pltpu.VMEM((DFF, D), BF16),
            pltpu.VMEM((D, D), I32),
            pltpu.VMEM((8, 6 * D), F32),
            pltpu.VMEM((NBLK, D // 2, T), I32),
            pltpu.VMEM((H, S // 2, 128), I32),
            pltpu.VMEM((S // QB, D // 2, QB), I32),
            pltpu.VMEM((NBLK, T, D), BF16),
            pltpu.VMEM((NBLK + 1, 4, T, 128), BF16),
            pltpu.VMEM((NBLK, T, D), F32),
            pltpu.VMEM((NBLK, 4, T, 128), BF16),
            pltpu.SemaphoreType.DMA((12,)),
        ],
        compiler_params=pltpu.CompilerParams(
            dimension_semantics=("arbitrary",), vmem_limit_bytes=100 * 1024 * 1024),
    )(c, A_x, w_mod, A_wqkv, A_wo, B_w1, B_w2)
```

```python
import functools
import jax
import jax.numpy as jnp
from jax import lax
import jax.experimental.pallas as pl
import jax.experimental.pallas.tpu as pltpu

S = 2048
D = 512
H = 32
DH = 16
DFF = 1792
T = 256
QB = 128
HB = QB // 2
NG = 4
NBLK = S // T
NKB = T // QB
LOG2E = 1.4426950408889634
QSCALE = 0.25 * LOG2E
NEG = -1e30
EPS = 1e-5
PG = [0.85, 40.0, 44.0, 8.0, 0.0]
P0 = [0.93, 60.0, 48.0, 12.0, 1.0]
PN = [0.7, 40.0, 44.0, 8.0, 0.0]
ORD = 'acdebfghABCD'
ORD0 = 'deWmcfabgh'
L0R = [0.0, 1.0, 0.9]
ORDN = 'abABCD'
L1R = [0.1, 0.9]
L2R = [0.95]
QW = 6
KCH = 64
CMAX = 128
NS = 3
DORD = '2103456789abc'
LR0 = 128
NSAT = 2
LR = 32
TIE = 1
F1R = 256
F2R = 128
NT = (((1,), (1,)), ((), ()))
F32 = jnp.float32
BF16 = jnp.bfloat16
I32 = jnp.int32


def _ln(xf, tie=None):
    mu = jnp.mean(xf, axis=-1, keepdims=True)
    if tie is not None:
        mu = jnp.where(tie[0], tie[1], mu)
    xc = xf - mu
    var = jnp.mean(xc * xc, axis=-1, keepdims=True)
    return xc * lax.rsqrt(var + EPS)


def _pk(v):
    return pltpu.bitcast(v.astype(BF16), I32)


def _up(v):
    return pltpu.bitcast(v, BF16)


def _dot(a, b):
    return jnp.dot(a, b, preferred_element_type=F32)


def _dot_nt(a, b):
    return lax.dot_general(a, b, NT, preferred_element_type=F32)


def _kernel(c_ref, x_hbm, wmod_hbm, wqkv_hbm, wo_hbm, w1_hbm, w2_hbm, o_ref,
            x_v, wmod_v, wqkv_v, wo_v, w1_v, w2_v, wqvt_v, mod_v, qt_v, k8_v, vt_v, ao_v, h_v, x1_v, h2_v,
            sems):
    i = pl.program_id(0)

    def cp(src, dst, k):
        return pltpu.make_async_copy(src, dst, sems.at[k])

    cp_moda = cp(wmod_hbm.at[:, 0:2 * D], wmod_v.at[:, 0:2 * D], 0)
    cp_x0 = cp(x_hbm.at[0, 0:T, :], x_v.at[0:T, :], 1)
    cp_wq = cp(wqkv_hbm.at[:, 0:D], wqkv_v.at[:, 0:D], 2)
    cp_x1 = cp(x_hbm.at[0, T:2 * T, :], x_v.at[T:2 * T, :], 3)
    cp_wk = cp(wqkv_hbm.at[:, D:2 * D], wqkv_v.at[:, D:2 * D], 4)
    cp_wv = cp(wqkv_hbm.at[:, 2 * D:3 * D], wqkv_v.at[:, 2 * D:3 * D], 5)
    cp_x2 = cp(x_hbm.at[0, 2 * T:3 * T, :], x_v.at[2 * T:3 * T, :], 6)
    cp_x3 = cp(x_hbm.at[0, 3 * T:4 * T, :], x_v.at[3 * T:4 * T, :], 7)
    cp_modb = cp(wmod_hbm.at[:, 2 * D:6 * D], wmod_v.at[:, 2 * D:6 * D], 8)
    cp_wo = cp(wo_hbm, wo_v, 9)
    cp_w1 = cp(w1_hbm, w1_v, 10)
    cp_w2 = cp(w2_hbm, w2_v, 11)
    cp_xr = cp(x_hbm.at[0, 4 * T:S, :], x_v.at[4 * T:S, :], 12)
    cps = [cp_moda, cp_x0, cp_wq, cp_x1, cp_wk, cp_wv, cp_x2, cp_x3, cp_modb, cp_wo, cp_w1, cp_w2, cp_xr]
    all_cp = [cps[int(ch, 16)] for ch in DORD]

    def silu_c():
        c = c_ref[...].astype(F32)
        sc = c * jax.nn.sigmoid(c)
        return jnp.broadcast_to(sc, (8, D)).astype(BF16)

    def modmm(lo, hi):
        mod_v[:, lo * D:hi * D] = _dot(silu_c(), wmod_v[:, lo * D:hi * D])

    def xrows(blk, r0, n, c0=0, c1=D):
        start = blk * T + r0
        if not isinstance(start, int):
            start = pl.multiple_of(start, n)
        return x_v[pl.ds(start, n), c0:c1]

    def step(kind):
        with jax.named_scope('st_' + kind):
            step_(kind)

    def step_(kind):
        first = kind == 'first'
        gen = kind == 'gen'
        if gen:
            qt_r = qt_v.at[pl.ds(i + 1, 2)]
            k8_r = k8_v.at[:, pl.ds(pl.multiple_of(i * (T // 2), T // 2), 3 * (T // 2)), :]
            vt_r = vt_v.at[pl.ds(i * NKB, 3 * NKB)]
            ao_r = ao_v.at[pl.ds(i, 2)]
            h_r = h_v.at[pl.ds(i + 2, 2)]
            x1_r = x1_v.at[pl.ds(i - 1, 2)]
            h2_r = h2_v.at[pl.ds(i - 1, 2)]
        else:
            qt_r, k8_r, vt_r, ao_r, h_r, x1_r, h2_r = qt_v, k8_v, vt_v, ao_v, h_v, x1_v, h2_v

        loads = [0, 0, 0, 0]
        run = [0, 0, 0, 0]

        def acct(n):
            m = min(range(4), key=lambda k: (loads[k], k))
            loads[m] += max(n, 2)
            run[m] = run[m] + 1 if n <= 2 else 0

        lane = lax.broadcasted_iota(I32, (KCH, 128), 1)
        low_of = {w: ((lane // w) % 2) == 0 for w in (64, 32, 16)}
        bb = lax.broadcasted_iota(I32, (QB, QB), 0)
        aa = lax.broadcasted_iota(I32, (QB, QB), 1)
        tri = bb > aa
        diag = (lax.broadcasted_iota(I32, (HB, 128), 0) // 8) == (lax.broadcasted_iota(I32, (HB, 128), 1) // DH)
        use_l = (lax.broadcasted_iota(I32, (HB - 8, 128), 1) // DH) > (lax.broadcasted_iota(I32, (HB - 8, 128), 0) // 8)

        st = {}

        def acc(key, val):
            st[key] = val if key not in st else val + st[key]
            if val.shape[0] >= QB:
                st['last'] = st[key]
            return st[key]

        def tie(rows):
            v = st.get('last')
            if v is None or not TIE:
                return None
            return (i < 0, v[0:rows, 0:1])

        def ln1_chunk(xblk, hidx, r0, xn=None):
            if xn is None:
                xn = _ln(xrows(xblk, r0, LR).astype(F32), tie(LR))
            h = (xn * (1.0 + mod_v[0:1, D:2 * D]) + mod_v[0:1, 0:D]).astype(BF16)
            for k in range(4):
                h_r[hidx, k, r0:r0 + xn.shape[0], :] = h[:, k * 128:(k + 1) * 128]

        def ln2_chunk(widx, r0):
            xn = _ln(x1_r[widx, r0:r0 + LR, :], tie(LR))
            h = (xn * (1.0 + mod_v[0:1, 4 * D:5 * D]) + mod_v[0:1, 3 * D:4 * D]).astype(BF16)
            for k in range(4):
                h2_r[widx, k, r0:r0 + LR, :] = h[:, k * 128:(k + 1) * 128]

        def ln1_tasks(xblk, hidx, j=None):
            rows = range(0, T, LR) if j is None else range(j * QB, (j + 1) * QB, LR)
            return [(functools.partial(ln1_chunk, xblk, hidx, r0), 0, 0) for r0 in rows]

        def ln2_tasks(widx, j, need=0):
            return [(functools.partial(ln2_chunk, widx, r0), 0, need) for r0 in range(j * QB, (j + 1) * QB, LR)]

        def k_tile(blk, j, g, k):
            r = acc(('k', blk, j, g), _dot(h_r[blk[0], k, j * QB:(j + 1) * QB, :],
                                           wqkv_v[k * 128:(k + 1) * 128, D + g * 128:D + (g + 1) * 128]))
            if k == 3:
                kb = _pk(r)
                for r0 in range(0, HB, KCH):
                    vs = [kb[r0:r0 + KCH]]
                    for w in (64, 32, 16):
                        nxt = []
                        for v in vs:
                            rv = pltpu.roll(v, w, 1)
                            nxt += [jnp.where(low_of[w], v, rv), jnp.where(low_of[w], rv, v)]
                        vs = nxt
                    for hh in range(8):
                        k8_r[g * 8 + hh, pl.ds(blk[2] * (T // 2) + j * HB + r0, KCH), :] = vs[hh]

        def q_tile(blk, j, r, k):
            w = _up(wqvt_v[r * 128:(r + 1) * 128, k * 128:(k + 1) * 128])
            res = acc(('q', blk, r, j), _dot_nt(w, h_r[blk[0], k, j * QB:(j + 1) * QB, :]))
            if k == 3:
                qt_r[blk[1], r * 128:(r + 1) * 128, j * QB:(j + 1) * QB] = _pk(res * QSCALE)

        def v_tile(blk, j, r, k):
            w = _up(wqvt_v[D // 2 + r * 128:D // 2 + (r + 1) * 128, k * 128:(k + 1) * 128])
            res = acc(('v', blk, r, j), _dot_nt(w, h_r[blk[0], k, j * QB:(j + 1) * QB, :]))
            if k == 3:
                vt_r[blk[2] * NKB + j, r * 128:(r + 1) * 128, :] = _pk(res)

        def proj_tasks(blk, j):
            kt = [(functools.partial(k_tile, blk, j, g, k), 8, 0) for g in range(NG) for k in range(4)]
            qt = [(functools.partial(q_tile, blk, j, r, k), 16, 0) for r in range(2) for k in range(4)]
            vt = [(functools.partial(v_tile, blk, j, r, k), 16, 0) for r in range(2) for k in range(4)]
            return kt, qt, vt

        def wo_tile(blk, j, n, k):
            y = acc(('y', blk[1], j, n), _dot(ao_r[blk[1], j * QB:(j + 1) * QB, k * 128:(k + 1) * 128],
                                              wo_v[k * 128:(k + 1) * 128, n * 128:(n + 1) * 128]))
            if k == 3:
                ga = mod_v[0:1, 2 * D + n * 128:2 * D + (n + 1) * 128]
                x1_r[blk[2], j * QB:(j + 1) * QB, n * 128:(n + 1) * 128] = (
                    xrows(blk[0], j * QB, QB, n * 128, (n + 1) * 128).astype(F32) + ga * y)

        def wo_tasks(blk, j, need=0):
            return [(functools.partial(wo_tile, blk, j, n, k), 8, need) for n in range(4) for k in range(4)]

        def f1_tile(widx, r, c, k):
            f = acc(('f1', r, c), _dot(h2_r[widx, k, r * F1R:(r + 1) * F1R, :],
                                       w1_v[k * 128:(k + 1) * 128, c * 128:(c + 1) * 128]))
            if k == 3:
                f = jnp.maximum(f, 0.0).astype(BF16)
                if F1R == T:
                    st['f', 0, c] = f[0:QB]
                    st['f', 1, c] = f[QB:]
                else:
                    st['f', r, c] = f

        def f2_tile(widx, n, r, c):
            if F2R == T:
                f = jnp.concatenate([st['f', 0, c], st['f', 1, c]], axis=0)
            else:
                f = st['f', r, c]
            z = acc(('z', n, r), _dot(f, w2_v[c * 128:(c + 1) * 128, n * 128:(n + 1) * 128]))
            if c == DFF // 128 - 1:
                gb = mod_v[0:1, 5 * D + n * 128:5 * D + (n + 1) * 128]
                x1 = x1_r[widx, r * F2R:(r + 1) * F2R, n * 128:(n + 1) * 128]
                o_ref[r * F2R:(r + 1) * F2R, n * 128:(n + 1) * 128] = (x1 + gb * z).astype(o_ref.dtype)

        def f1_tasks(widx, r):
            return [(functools.partial(f1_tile, widx, r, c, k), F1R // 16, 0)
                    for c in range(DFF // 128) for k in range(4)]

        def f2_tasks(widx, r):
            return [(functools.partial(f2_tile, widx, n, r, c), F2R // 16, 0)
                    for n in range(4) for c in range(DFF // 128)]

        def ffn_groups(groups, widx):
            groups['A'] = f1_tasks(widx, 0)
            groups['B'] = f1_tasks(widx, 1) if F1R != T else []
            groups['C'] = f2_tasks(widx, 0)
            groups['D'] = f2_tasks(widx, 1) if F2R != T else []

        def lhs(ib, head, j, has_first, has_mid):
            kl = (ib[1] * NKB + j) * HB
            if has_first:
                parts = [k8_r[head, pl.ds(kl, 8), :],
                         jnp.where(use_l, k8_r[head, pl.ds(kl + 8, HB - 8), :], k8_r[head, pl.ds(kl - 2 * HB, HB - 8), :]),
                         k8_r[head, pl.ds(kl - HB - 8, 8), :]]
            else:
                parts = [k8_r[head, pl.ds(kl, HB), :]]
            if has_mid:
                parts.append(k8_r[head, pl.ds(kl - HB, HB), :])
            return _up(jnp.concatenate(parts, axis=0) if len(parts) > 1 else parts[0])

        def qk_rows(has_first, has_mid):
            return (9 if has_first else 8) + (8 if has_mid else 0)

        def stage_a(g, hh, j, has_first, has_mid, ib):
            kwin = lhs(ib, g * 8 + hh, j, has_first, has_mid)
            r0 = g * 64 + hh * 8
            qh = qt_r[ib[0], r0:r0 + 8, j * QB:(j + 1) * QB]
            w = _up(jnp.where(diag, jnp.concatenate([qh] * 8, axis=0), 0))
            s_t = _dot(kwin, w)
            if has_first:
                sm = jnp.where(tri, s_t[DH:QB + DH], s_t[0:QB])
                rest = s_t[QB + DH:]
            else:
                sm = jnp.where(tri, NEG, s_t[0:QB])
                rest = s_t[QB:]
            s = jnp.concatenate([sm, rest], axis=0) if has_mid else sm
            m = jnp.max(s, axis=0, keepdims=True)
            st['s', g, hh, j] = (s, m)

        def pv_tiles(g, hh, j, has_first, has_mid, ib):
            qb = ib[1] * NKB + j
            r0 = g * 64 + hh * 8
            key = ('p', g, hh, j)

            def prep():
                s, m = st.pop(('s', g, hh, j))
                p = jnp.exp2(s - m)
                st[key] = (p, jnp.sum(p, axis=0, keepdims=True))

            def tile(which, is_first, is_last):
                if is_first:
                    prep()
                p, l = st[key]
                pm = p[0:QB]
                if which == 'L':
                    pp = jnp.where(tri, 0.0, pm) if has_first else pm
                    vv = vt_r[qb, r0:r0 + 8, :]
                elif which == 'M':
                    pp = p[QB:2 * QB]
                    vv = vt_r[qb - 1, r0:r0 + 8, :]
                else:
                    pp = jnp.where(tri, pm, 0.0)
                    vv = vt_r[qb - 2, r0:r0 + 8, :]
                ot = acc(('o', ib[1], g, hh, j), _dot(_up(vv), pp.astype(BF16)))
                if is_last:
                    st['on', g, j, hh] = ot * (1.0 / l)
                    if hh == 7:
                        og = jnp.concatenate([st['on', g, j, q] for q in range(8)], axis=0)
                        ao_r[ib[2], j * QB:(j + 1) * QB, g * 128:(g + 1) * 128] = og.T.astype(BF16)

            kinds = ['L'] + (['M'] if has_mid else []) + (['F'] if has_first else [])
            return [functools.partial(tile, w, q == 0, q == len(kinds) - 1) for q, w in enumerate(kinds)]

        def schedule(units, dense, params, gated=(), uneed=None, barrier=None):
            frac, lead, lag, maxin, PACE = params
            gated = list(gated)
            n = len(units)
            ucost = [qk_rows(u[3], u[4]) + 1 + u[3] + u[4] for u in units]
            dtot = sum(max(c, 2) for _, c, _ in dense + gated if c)
            tot = (dtot + sum(qk_rows(u[3], u[4]) + 2 * (1 + u[3] + u[4]) for u in units)) / 4.0
            base = min(loads)
            rate = frac * tot / max(n, 1)
            reserve = (1.0 - frac) * 4.0 * tot
            drem = dtot
            credit = lead
            nq = 0
            npv = 0
            pvq = []
            qk_time = {}
            nd = 0
            while nq < n or npv < n or dense or gated:
                now = min(loads) - base
                m = min(range(4), key=lambda k: (loads[k], k))
                pv_ok = npv < nq and now >= qk_time[npv] + lag
                qk_can = nq < n and nq - npv < maxin and (uneed is None or nd >= uneed[nq])
                if PACE:
                    spacing = max(drem - reserve, 0.0) * ucost[nq] / sum(ucost[nq:]) if nq < n else 0.0
                    qk_due = qk_can and credit >= spacing
                else:
                    qk_due = qk_can and now >= nq * rate - lead
                quiet = any(t[0] is barrier for t in dense[:QW]) and dense[0][2] <= npv
                if gated and npv >= gated[0][2]:
                    choice = 'g'
                elif quiet:
                    choice = 'd'
                elif pv_ok and run[m] < 2:
                    choice = 'pv'
                elif qk_due:
                    choice = 'qk'
                elif dense and dense[0][2] <= npv:
                    choice = 'd'
                elif qk_can:
                    choice = 'qk'
                else:
                    choice = 'pv'
                if choice == 'pv':
                    if not pvq:
                        pvq = pv_tiles(*units[npv])
                    fn = pvq.pop(0)
                    fn()
                    acct(1)
                    if not pvq:
                        npv += 1
                elif choice == 'qk':
                    qk_time[nq] = now
                    if PACE:
                        credit = min(credit - spacing, CMAX)
                    stage_a(*units[nq])
                    acct(qk_rows(units[nq][3], units[nq][4]))
                    nq += 1
                else:
                    fn, c, _ = (dense if choice == 'd' else gated).pop(0)
                    nd += choice == 'd'
                    fn()
                    if c:
                        acct(c)
                        drem -= max(c, 2)
                        credit += max(c, 2)

        def mk_units(ib, flags):
            return [(g, hh, j) + flags[j] + (ib,) for j in range(NKB) for g in range(NG) for hh in range(8)]

        def mod_tasks(lo, hi):
            def t(q):
                mod_v[:, q * 128:(q + 1) * 128] = _dot(silu_c(), wmod_v[:, q * 128:(q + 1) * 128])
            return [(functools.partial(t, q), 8, 0) for q in range(lo * 4, hi * 4)]

        def build(order, groups):
            dense = []
            ends = {}
            for ch in order:
                dense = dense + groups[ch]
                ends[ch] = len(dense)
            return dense, ends

        def sprinkle(dense, extras):
            ins = []
            for tasks, lo, hi in extras:
                hi = max(hi, lo)
                for q, t in enumerate(tasks):
                    ins.append((lo + (hi - lo) * (q + 0.5) / len(tasks), t))
            ins.sort(key=lambda e: e[0])
            out = []
            for pos, t in enumerate(dense):
                while ins and ins[0][0] <= pos:
                    out.append(ins.pop(0)[1])
                out.append(t)
            return out + [e[1] for e in ins]

        def proj_groups(groups, blk):
            groups['c'], groups['d'], groups['e'] = proj_tasks(blk, 0)
            groups['f'], groups['g'], groups['h'] = proj_tasks(blk, 1)

        full = [(True, True)] * NKB
        if first:
            for c_ in all_cp[:NS]:
                c_.start()
            cp_x0.wait()
            if NSAT == 1:
                for c_ in all_cp[NS:]:
                    c_.start()
            xn0 = [_ln(x_v[r0:r0 + LR0, :].astype(F32)) for r0 in range(0, T, LR0)]
            cp_wq.wait()
            if NSAT == 2:
                for c_ in all_cp[NS:]:
                    c_.start()
            wqvt_v[0:D // 2, :] = _pk(wqkv_v[:, 0:D].astype(F32).T)
            cp_moda.wait()
            if NSAT == 3:
                for c_ in all_cp[NS:]:
                    c_.start()
            modmm(0, 2)
            for q, r0 in enumerate(range(0, T, LR0)):
                ln1_chunk(0, 0, r0, xn0[q])
            cp_x1.wait()
            pr = [[proj_tasks((b, b, b), j) for j in range(NKB)] for b in range(3)]
            for fn, _, _ in ln1_tasks(1, 1):
                fn()
            for b in range(2):
                for j in range(NKB):
                    for fn, _, _ in pr[b][j][1]:
                        fn()
            cp_wk.wait()
            cp_wv.wait()
            cp_x2.wait()
            wqvt_v[D // 2:D, :] = _pk(wqkv_v[:, 2 * D:3 * D].astype(F32).T)
            for fn, c, _ in pr[0][0][0] + pr[0][0][2]:
                fn()
                acct(c)
            dense = []
            marks = []
            for b, j in ((0, 1), (1, 0), (1, 1)):
                dense += pr[b][j][0] + pr[b][j][2]
                marks.append(len(dense))
            groups = {}
            proj_groups(groups, (2, 2, 2))

            def waits():
                cp_x3.wait()
                cp_modb.wait()
                cp_wo.wait()

            groups['W'] = [(waits, 0, 0)]
            groups['m'] = mod_tasks(2, 6)
            groups['a'] = wo_tasks((0, 0, 0), 0, NG * 8)
            groups['b'] = wo_tasks((0, 0, 0), 1, 2 * NG * 8)
            n0 = len(dense)
            rest, ends = build(ORD0, groups)
            n = len(rest)
            rest = sprinkle(rest, [(ln1_tasks(3, 3), ends['W'] + L0R[0] * (n - ends['W']), ends['W'] + L0R[1] * (n - ends['W'])),
                                   (ln2_tasks(0, 0), ends['a'], ends['a'] + L0R[2] * (n - ends['a'])),
                                   (ln2_tasks(0, 1), ends['b'], ends['b'] + L0R[2] * (n - ends['b']))])
            l2 = ln1_tasks(2, 2)
            dense = sprinkle(dense, [(l2, 0, n0)]) + rest
            marks = [mk + sum(1 for q in range(len(l2)) if n0 * (q + 0.5) / len(l2) <= mk) for mk in marks]
            u0 = mk_units((0, 0, 0), [(False, False), (False, True)])
            u1 = mk_units((1, 1, 1), full)
            uneed = [0] * 32 + [marks[0]] * 32 + [marks[1]] * 32 + [marks[2]] * 32
            schedule(u0 + u1, dense, P0, uneed=uneed, barrier=waits)
            cp_w1.wait()
            cp_w2.wait()
            cp_xr.wait()
        elif gen:
            groups = {'a': wo_tasks((i, 0, 1), 0), 'b': wo_tasks((i, 0, 1), 1)}
            ffn_groups(groups, 0)
            proj_groups(groups, (0, 1, 2))
            dense, ends = build(ORD, groups)
            n = len(dense)
            dense = sprinkle(dense, [(ln1_tasks(jnp.minimum(i + 3, NBLK - 1), 1), L1R[0] * n, L1R[1] * n),
                                     (ln2_tasks(1, 0), ends['a'], L2R[0] * n), (ln2_tasks(1, 1), ends['b'], L2R[0] * n)])
            schedule(mk_units((0, 1, 1), full), dense, PG)
        elif kind == 'noproj':
            lb = NBLK - 1
            groups = {'a': wo_tasks((lb - 1,) * 3, 0), 'b': wo_tasks((lb - 1,) * 3, 1)}
            ffn_groups(groups, lb - 2)
            dense, ends = build(ORDN, groups)
            n = len(dense)
            dense = sprinkle(dense, [(ln2_tasks(lb - 1, 0), ends['a'], L2R[0] * n),
                                     (ln2_tasks(lb - 1, 1), ends['b'], L2R[0] * n)])
            gated = []
            for j in range(NKB):
                need = (j + 1) * NG * 8
                gated += wo_tasks((lb,) * 3, j, need) + ln2_tasks(lb, j, need)
            schedule(mk_units((lb,) * 3, full), dense, PN, gated)
        else:
            groups = {}
            ffn_groups(groups, i - 1)
            schedule([], build('ABCD', groups)[0], PG)

    variants = [
        (jnp.logical_and(i > 0, i < NBLK - 2), 'gen'),
        (i == 0, 'first'),
        (i == NBLK - 2, 'noproj'),
        (i > NBLK - 2, 'last'),
    ]
    for cond, kind in variants:
        pl.when(cond)(functools.partial(step, kind))


@jax.jit
def pallas_adaLN_cond__sliding_block__dense_activation_relu__prompt_kernel(A_x, A_wqkv, A_wo, B_x, B_w1, B_w2, c, w_mod):
    any_spec = pl.BlockSpec(memory_space=pl.ANY)
    return pl.pallas_call(
        _kernel,
        grid=(NBLK + 1,),
        in_specs=[
            pl.BlockSpec((1, D), lambda i: (0, 0)),
            any_spec, any_spec, any_spec, any_spec, any_spec, any_spec,
        ],
        out_specs=pl.BlockSpec((None, T, D), lambda i: (0, jnp.maximum(i - 1, 0), 0)),
        out_shape=jax.ShapeDtypeStruct((1, S, D), BF16),
        scratch_shapes=[
            pltpu.VMEM((S, D), BF16),
            pltpu.VMEM((D, 6 * D), BF16),
            pltpu.VMEM((D, 3 * D), BF16),
            pltpu.VMEM((D, D), BF16),
            pltpu.VMEM((D, DFF), BF16),
            pltpu.VMEM((DFF, D), BF16),
            pltpu.VMEM((D, D), I32),
            pltpu.VMEM((8, 6 * D), F32),
            pltpu.VMEM((NBLK, D // 2, T), I32),
            pltpu.VMEM((H, S // 2, 128), I32),
            pltpu.VMEM((S // QB, D // 2, QB), I32),
            pltpu.VMEM((NBLK, T, D), BF16),
            pltpu.VMEM((NBLK + 1, 4, T, 128), BF16),
            pltpu.VMEM((NBLK, T, D), F32),
            pltpu.VMEM((NBLK, 4, T, 128), BF16),
            pltpu.SemaphoreType.DMA((13,)),
        ],
        compiler_params=pltpu.CompilerParams(
            dimension_semantics=("arbitrary",), vmem_limit_bytes=100 * 1024 * 1024),
    )(c, A_x, w_mod, A_wqkv, A_wo, B_w1, B_w2)
```

```python
import functools
import jax
import jax.numpy as jnp
from jax import lax
import jax.experimental.pallas as pl
import jax.experimental.pallas.tpu as pltpu

S = 2048
D = 512
H = 32
DH = 16
DFF = 1792
T = 256
QB = 128
HB = QB // 2
NG = 4
NBLK = S // T
NKB = T // QB
LOG2E = 1.4426950408889634
QSCALE = 0.25 * LOG2E
NEG = -1e30
EPS = 1e-5
PG = [0.95, 10.0, 40.0, 7.0, 0.0]
P0 = [0.93, 0.0, 28.0, 10.0, 1.0]
PN = [0.65, 20.0, 36.0, 8.0, 1.0]
ORD = 'acdebfghABCD'
ORD0 = 'dehWmcfabg'
L0R = [0.0, 0.8, 0.8]
ORDN = 'aAbCD'
L1R = [0.1, 0.9]
L2R = [1.0]
QW = 3
KCH = 64
L2N = [0.5]
CMN = 16
HALF = 2
CMAX = 64
NS = 3
DORD = '2103456789abc'
LR0 = 128
NSAT = 2
LR = 32
TIE = 1
F1R = 256
F2R = 128
NT = (((1,), (1,)), ((), ()))
F32 = jnp.float32
BF16 = jnp.bfloat16
I32 = jnp.int32


def _ln(xf, tie=None):
    mu = jnp.mean(xf, axis=-1, keepdims=True)
    if tie is not None:
        mu = jnp.where(tie[0], tie[1], mu)
    xc = xf - mu
    var = jnp.mean(xc * xc, axis=-1, keepdims=True)
    return xc * lax.rsqrt(var + EPS)


def _pk(v):
    return pltpu.bitcast(v.astype(BF16), I32)


def _up(v):
    return pltpu.bitcast(v, BF16)


def _dot(a, b):
    return jnp.dot(a, b, preferred_element_type=F32)


def _dot_nt(a, b):
    return lax.dot_general(a, b, NT, preferred_element_type=F32)


def _kernel(c_hbm, x_hbm, wmod_hbm, wqkv_hbm, wo_hbm, w1_hbm, w2_hbm, o_ref,
            x_v, wmod_v, wqkv_v, wo_v, w1_v, w2_v, wqvt_v, mod_v, qt_v, k8_v, vt_v, ao_v, h_v, x1_v, h2_v,
            c_ref, sems):
    i = pl.program_id(0)

    def cp(src, dst, k):
        return pltpu.make_async_copy(src, dst, sems.at[k])

    cp_moda = cp(wmod_hbm.at[:, 0:2 * D], wmod_v.at[:, 0:2 * D], 0)
    cp_x0 = cp(x_hbm.at[0, 0:T, :], x_v.at[0:T, :], 1)
    cp_wq = cp(wqkv_hbm.at[:, 0:D], wqkv_v.at[:, 0:D], 2)
    cp_x1 = cp(x_hbm.at[0, T:2 * T, :], x_v.at[T:2 * T, :], 3)
    cp_wk = cp(wqkv_hbm.at[:, D:2 * D], wqkv_v.at[:, D:2 * D], 4)
    cp_wv = cp(wqkv_hbm.at[:, 2 * D:3 * D], wqkv_v.at[:, 2 * D:3 * D], 5)
    cp_x2 = cp(x_hbm.at[0, 2 * T:3 * T, :], x_v.at[2 * T:3 * T, :], 6)
    cp_x3 = cp(x_hbm.at[0, 3 * T:4 * T, :], x_v.at[3 * T:4 * T, :], 7)
    cp_modb = cp(wmod_hbm.at[:, 2 * D:6 * D], wmod_v.at[:, 2 * D:6 * D], 8)
    cp_wo = cp(wo_hbm, wo_v, 9)
    cp_w1 = cp(w1_hbm, w1_v, 10)
    cp_w2 = cp(w2_hbm, w2_v, 11)
    cp_xr = cp(x_hbm.at[0, 4 * T:S, :], x_v.at[4 * T:S, :], 12)
    cp_c = cp(c_hbm, c_ref, 13)
    cps = [cp_moda, cp_x0, cp_wq, cp_x1, cp_wk, cp_wv, cp_x2, cp_x3, cp_modb, cp_wo, cp_w1, cp_w2, cp_xr]
    all_cp = [cps[int(ch, 16)] for ch in DORD]

    def silu_c():
        c = c_ref[...].astype(F32)
        sc = c * jax.nn.sigmoid(c)
        return jnp.broadcast_to(sc, (8, D)).astype(BF16)

    def modmm(lo, hi):
        mod_v[:, lo * D:hi * D] = _dot(silu_c(), wmod_v[:, lo * D:hi * D])

    def xrows(blk, r0, n, c0=0, c1=D):
        start = blk * T + r0
        if not isinstance(start, int):
            start = pl.multiple_of(start, n)
        return x_v[pl.ds(start, n), c0:c1]

    def step(kind):
        with jax.named_scope('st_' + kind):
            step_(kind)

    def step_(kind):
        first = kind == 'first'
        gen = kind == 'gen'
        if gen:
            qt_r = qt_v.at[pl.ds(i + 1, 2)]
            k8_r = k8_v.at[:, pl.ds(pl.multiple_of(i * (T // 2), T // 2), 3 * (T // 2)), :]
            vt_r = vt_v.at[pl.ds(i * NKB, 3 * NKB)]
            ao_r = ao_v.at[pl.ds(i, 2)]
            h_r = h_v.at[pl.ds(i + 2, 2)]
            x1_r = x1_v.at[pl.ds(i - 1, 2)]
            h2_r = h2_v.at[pl.ds(i - 1, 2)]
        else:
            qt_r, k8_r, vt_r, ao_r, h_r, x1_r, h2_r = qt_v, k8_v, vt_v, ao_v, h_v, x1_v, h2_v

        loads = [0, 0, 0, 0]
        run = [0, 0, 0, 0]

        def acct(n):
            m = min(range(4), key=lambda k: (loads[k], k))
            loads[m] += max(n, 2)
            run[m] = run[m] + 1 if n <= 2 else 0

        lane = lax.broadcasted_iota(I32, (KCH, 128), 1)
        low_of = {w: ((lane // w) % 2) == 0 for w in (64, 32, 16)}
        bb = lax.broadcasted_iota(I32, (QB, QB), 0)
        aa = lax.broadcasted_iota(I32, (QB, QB), 1)
        tri = bb > aa
        diag = (lax.broadcasted_iota(I32, (HB, 128), 0) // 8) == (lax.broadcasted_iota(I32, (HB, 128), 1) // DH)
        use_l = (lax.broadcasted_iota(I32, (HB - 8, 128), 1) // DH) > (lax.broadcasted_iota(I32, (HB - 8, 128), 0) // 8)

        st = {}

        def acc(key, val):
            st[key] = val if key not in st else val + st[key]
            if val.shape[0] >= QB:
                st['last'] = st[key]
            return st[key]

        def tie(rows):
            v = st.get('last')
            if v is None or not TIE:
                return None
            return (i < 0, v[0:rows, 0:1])

        def ln1_chunk(xblk, hidx, r0, xn=None):
            if xn is None:
                xn = _ln(xrows(xblk, r0, LR).astype(F32), tie(LR))
            h = (xn * (1.0 + mod_v[0:1, D:2 * D]) + mod_v[0:1, 0:D]).astype(BF16)
            for k in range(4):
                h_r[hidx, k, r0:r0 + xn.shape[0], :] = h[:, k * 128:(k + 1) * 128]

        def ln2_chunk(widx, r0):
            xn = _ln(x1_r[widx, r0:r0 + LR, :], tie(LR))
            h = (xn * (1.0 + mod_v[0:1, 4 * D:5 * D]) + mod_v[0:1, 3 * D:4 * D]).astype(BF16)
            for k in range(4):
                h2_r[widx, k, r0:r0 + LR, :] = h[:, k * 128:(k + 1) * 128]

        def ln1_tasks(xblk, hidx, j=None):
            rows = range(0, T, LR) if j is None else range(j * QB, (j + 1) * QB, LR)
            return [(functools.partial(ln1_chunk, xblk, hidx, r0), 0, 0) for r0 in rows]

        def ln2_tasks(widx, j, need=0):
            return [(functools.partial(ln2_chunk, widx, r0), 0, need) for r0 in range(j * QB, (j + 1) * QB, LR)]

        def k_tile(blk, j, g, k):
            r = acc(('k', blk, j, g), _dot(h_r[blk[0], k, j * QB:(j + 1) * QB, :],
                                           wqkv_v[k * 128:(k + 1) * 128, D + g * 128:D + (g + 1) * 128]))
            if k == 3:
                kb = _pk(r)
                for r0 in range(0, HB, KCH):
                    vs = [kb[r0:r0 + KCH]]
                    for w in (64, 32, 16):
                        nxt = []
                        for v in vs:
                            rv = pltpu.roll(v, w, 1)
                            nxt += [jnp.where(low_of[w], v, rv), jnp.where(low_of[w], rv, v)]
                        vs = nxt
                    for hh in range(8):
                        k8_r[g * 8 + hh, pl.ds(blk[2] * (T // 2) + j * HB + r0, KCH), :] = vs[hh]

        def q_tile(blk, j, r, k):
            w = _up(wqvt_v[r * 128:(r + 1) * 128, k * 128:(k + 1) * 128])
            res = acc(('q', blk, r, j), _dot_nt(w, h_r[blk[0], k, j * QB:(j + 1) * QB, :]))
            if k == 3:
                qt_r[blk[1], r * 128:(r + 1) * 128, j * QB:(j + 1) * QB] = _pk(res * QSCALE)

        def v_tile(blk, j, r, k):
            w = _up(wqvt_v[D // 2 + r * 128:D // 2 + (r + 1) * 128, k * 128:(k + 1) * 128])
            res = acc(('v', blk, r, j), _dot_nt(w, h_r[blk[0], k, j * QB:(j + 1) * QB, :]))
            if k == 3:
                vt_r[blk[2] * NKB + j, r * 128:(r + 1) * 128, :] = _pk(res)

        def proj_tasks(blk, j):
            kt = [(functools.partial(k_tile, blk, j, g, k), 8, 0) for g in range(NG) for k in range(4)]
            qt = [(functools.partial(q_tile, blk, j, r, k), 16, 0) for r in range(2) for k in range(4)]
            vt = [(functools.partial(v_tile, blk, j, r, k), 16, 0) for r in range(2) for k in range(4)]
            return kt, qt, vt

        def wo_tile(blk, j, n, k):
            y = acc(('y', blk[1], j, n), _dot(ao_r[blk[1], j * QB:(j + 1) * QB, k * 128:(k + 1) * 128],
                                              wo_v[k * 128:(k + 1) * 128, n * 128:(n + 1) * 128]))
            if k == 3:
                ga = mod_v[0:1, 2 * D + n * 128:2 * D + (n + 1) * 128]
                x1_r[blk[2], j * QB:(j + 1) * QB, n * 128:(n + 1) * 128] = (
                    xrows(blk[0], j * QB, QB, n * 128, (n + 1) * 128).astype(F32) + ga * y)

        def wo_tasks(blk, j, need=0):
            return [(functools.partial(wo_tile, blk, j, n, k), 8, need) for n in range(4) for k in range(4)]

        def f1_tile(widx, r, c, k):
            f = acc(('f1', r, c), _dot(h2_r[widx, k, r * F1R:(r + 1) * F1R, :],
                                       w1_v[k * 128:(k + 1) * 128, c * 128:(c + 1) * 128]))
            if k == 3:
                f = jnp.maximum(f, 0.0).astype(BF16)
                if F1R == T:
                    st['f', 0, c] = f[0:QB]
                    st['f', 1, c] = f[QB:]
                else:
                    st['f', r, c] = f

        def f2_tile(widx, n, r, c):
            if F2R == T:
                f = jnp.concatenate([st['f', 0, c], st['f', 1, c]], axis=0)
            else:
                f = st['f', r, c]
            z = acc(('z', n, r), _dot(f, w2_v[c * 128:(c + 1) * 128, n * 128:(n + 1) * 128]))
            if c == DFF // 128 - 1:
                gb = mod_v[0:1, 5 * D + n * 128:5 * D + (n + 1) * 128]
                x1 = x1_r[widx, r * F2R:(r + 1) * F2R, n * 128:(n + 1) * 128]
                o_ref[r * F2R:(r + 1) * F2R, n * 128:(n + 1) * 128] = (x1 + gb * z).astype(o_ref.dtype)

        def f1_tasks(widx, r):
            return [(functools.partial(f1_tile, widx, r, c, k), F1R // 16, 0)
                    for c in range(DFF // 128) for k in range(4)]

        def f2_tasks(widx, r):
            return [(functools.partial(f2_tile, widx, n, r, c), F2R // 16, 0)
                    for n in range(4) for c in range(DFF // 128)]

        def ffn_groups(groups, widx):
            groups['A'] = f1_tasks(widx, 0)
            groups['B'] = f1_tasks(widx, 1) if F1R != T else []
            groups['C'] = f2_tasks(widx, 0)
            groups['D'] = f2_tasks(widx, 1) if F2R != T else []

        def lhs(ib, head, j, has_first, has_mid):
            kl = (ib[1] * NKB + j) * HB
            if has_first:
                parts = [k8_r[head, pl.ds(kl, 8), :],
                         jnp.where(use_l, k8_r[head, pl.ds(kl + 8, HB - 8), :], k8_r[head, pl.ds(kl - 2 * HB, HB - 8), :]),
                         k8_r[head, pl.ds(kl - HB - 8, 8), :]]
            else:
                parts = [k8_r[head, pl.ds(kl, HB), :]]
            if has_mid:
                parts.append(k8_r[head, pl.ds(kl - HB, HB), :])
            return _up(jnp.concatenate(parts, axis=0) if len(parts) > 1 else parts[0])

        def qk_rows(has_first, has_mid):
            return (9 if has_first else 8) + (8 if has_mid else 0)

        def stage_a(g, hh, j, has_first, has_mid, ib):
            kwin = lhs(ib, g * 8 + hh, j, has_first, has_mid)
            r0 = g * 64 + hh * 8
            qh = qt_r[ib[0], r0:r0 + 8, j * QB:(j + 1) * QB]
            w = _up(jnp.where(diag, jnp.concatenate([qh] * 8, axis=0), 0))
            s_t = _dot(kwin, w)
            if has_first:
                sm = jnp.where(tri, s_t[DH:QB + DH], s_t[0:QB])
                rest = s_t[QB + DH:]
            else:
                sm = jnp.where(tri, NEG, s_t[0:QB])
                rest = s_t[QB:]
            if HALF and has_mid:
                st['s', g, hh, j] = (sm, jnp.max(sm, axis=0, keepdims=True), rest, jnp.max(rest, axis=0, keepdims=True))
                return
            s = jnp.concatenate([sm, rest], axis=0) if has_mid else sm
            m = jnp.max(s, axis=0, keepdims=True)
            st['s', g, hh, j] = (s, m)

        def pv_tiles(g, hh, j, has_first, has_mid, ib):
            qb = ib[1] * NKB + j
            r0 = g * 64 + hh * 8
            key = ('p', g, hh, j)

            half = HALF and has_mid

            def prep():
                if half:
                    s1, m1, s2, m2 = st.pop(('s', g, hh, j))
                    p1 = jnp.exp2(s1 - m1)
                    p2 = jnp.exp2(s2 - m2)
                    m = jnp.maximum(m1, m2)
                    a1 = jnp.exp2(m1 - m)
                    a2 = jnp.exp2(m2 - m)
                    if HALF == 1:
                        l = a1 * jnp.sum(p1, axis=0, keepdims=True) + a2 * jnp.sum(p2, axis=0, keepdims=True)
                    else:
                        l8 = a1 * jnp.sum(p1.reshape(QB // 8, 8, QB), axis=0) + a2 * jnp.sum(p2.reshape(QB // 8, 8, QB), axis=0)
                        l = jnp.sum(l8, axis=0, keepdims=True)
                    st[key] = (p1, p2, l, a1, a2)
                    return
                s, m = st.pop(('s', g, hh, j))
                p = jnp.exp2(s - m)
                st[key] = (p[0:QB], p[QB:], jnp.sum(p, axis=0, keepdims=True), None, None)

            def tile(which, is_first, is_last):
                if is_first:
                    prep()
                pm, p2, l, a1, a2 = st[key]
                if which == 'L':
                    pp = jnp.where(tri, 0.0, pm) if has_first else pm
                    vv = vt_r[qb, r0:r0 + 8, :]
                elif which == 'M':
                    pp = p2
                    vv = vt_r[qb - 1, r0:r0 + 8, :]
                else:
                    pp = jnp.where(tri, pm, 0.0)
                    vv = vt_r[qb - 2, r0:r0 + 8, :]
                okey = ('o', ib[1], g, hh, j, half and which == 'M')
                ot = acc(okey, _dot(_up(vv), pp.astype(BF16)))
                if is_last:
                    if half:
                        inv = 1.0 / l
                        st['on', g, j, hh] = (st['o', ib[1], g, hh, j, False] * (a1 * inv)
                                              + st['o', ib[1], g, hh, j, True] * (a2 * inv))
                    else:
                        st['on', g, j, hh] = ot * (1.0 / l)
                    if hh == 7:
                        og = jnp.concatenate([st['on', g, j, q] for q in range(8)], axis=0)
                        ao_r[ib[2], j * QB:(j + 1) * QB, g * 128:(g + 1) * 128] = og.T.astype(BF16)

            kinds = ['L'] + (['M'] if has_mid else []) + (['F'] if has_first else [])
            return [functools.partial(tile, w, q == 0, q == len(kinds) - 1) for q, w in enumerate(kinds)]

        def schedule(units, dense, params, gated=(), uneed=None, barrier=None):
            frac, lead, lag, maxin, PACE = params
            gated = list(gated)
            n = len(units)
            ucost = [qk_rows(u[3], u[4]) + 1 + u[3] + u[4] for u in units]
            dtot = sum(max(c, 2) for _, c, _ in dense + gated if c)
            tot = (dtot + sum(qk_rows(u[3], u[4]) + 2 * (1 + u[3] + u[4]) for u in units)) / 4.0
            base = min(loads)
            rate = frac * tot / max(n, 1)
            reserve = (1.0 - frac) * 4.0 * tot
            drem = dtot
            credit = lead
            nq = 0
            npv = 0
            pvq = []
            qk_time = {}
            nd = 0
            while nq < n or npv < n or dense or gated:
                now = min(loads) - base
                m = min(range(4), key=lambda k: (loads[k], k))
                pv_ok = npv < nq and now >= qk_time[npv] + lag
                qk_can = nq < n and nq - npv < maxin and (uneed is None or nd >= uneed[nq])
                if PACE:
                    spacing = max(drem - reserve, 0.0) * ucost[nq] / sum(ucost[nq:]) if nq < n else 0.0
                    qk_due = qk_can and credit >= spacing
                else:
                    qk_due = qk_can and now >= nq * rate - lead
                quiet = any(t[0] is barrier for t in dense[:QW]) and dense[0][2] <= npv
                if gated and npv >= gated[0][2]:
                    choice = 'g'
                elif quiet:
                    choice = 'd'
                elif pv_ok and run[m] < 2:
                    choice = 'pv'
                elif qk_due:
                    choice = 'qk'
                elif dense and dense[0][2] <= npv:
                    choice = 'd'
                elif qk_can:
                    choice = 'qk'
                else:
                    choice = 'pv'
                if choice == 'pv':
                    if not pvq:
                        pvq = pv_tiles(*units[npv])
                    fn = pvq.pop(0)
                    fn()
                    acct(1)
                    if not pvq:
                        npv += 1
                elif choice == 'qk':
                    qk_time[nq] = now
                    if PACE:
                        credit = min(credit - spacing, CMAX if first else CMN)
                    stage_a(*units[nq])
                    acct(qk_rows(units[nq][3], units[nq][4]))
                    nq += 1
                else:
                    fn, c, _ = (dense if choice == 'd' else gated).pop(0)
                    nd += choice == 'd'
                    fn()
                    if c:
                        acct(c)
                        drem -= max(c, 2)
                        credit += max(c, 2)

        def mk_units(ib, flags):
            return [(g, hh, j) + flags[j] + (ib,) for j in range(NKB) for g in range(NG) for hh in range(8)]

        def mod_tasks(lo, hi):
            def t(q):
                mod_v[:, q * 128:(q + 1) * 128] = _dot(silu_c(), wmod_v[:, q * 128:(q + 1) * 128])
            return [(functools.partial(t, q), 8, 0) for q in range(lo * 4, hi * 4)]

        def build(order, groups):
            dense = []
            ends = {}
            for ch in order:
                dense = dense + groups[ch]
                ends[ch] = len(dense)
            return dense, ends

        def sprinkle(dense, extras):
            ins = []
            for tasks, lo, hi in extras:
                hi = max(hi, lo)
                for q, t in enumerate(tasks):
                    ins.append((lo + (hi - lo) * (q + 0.5) / len(tasks), t))
            ins.sort(key=lambda e: e[0])
            out = []
            for pos, t in enumerate(dense):
                while ins and ins[0][0] <= pos:
                    out.append(ins.pop(0)[1])
                out.append(t)
            return out + [e[1] for e in ins]

        def proj_groups(groups, blk):
            groups['c'], groups['d'], groups['e'] = proj_tasks(blk, 0)
            groups['f'], groups['g'], groups['h'] = proj_tasks(blk, 1)

        full = [(True, True)] * NKB
        if first:
            for c_ in all_cp[:NS]:
                c_.start()
            cp_c.start()
            cp_x0.wait()
            if NSAT == 1:
                for c_ in all_cp[NS:]:
                    c_.start()
            xn0 = [_ln(x_v[r0:r0 + LR0, :].astype(F32)) for r0 in range(0, T, LR0)]
            cp_wq.wait()
            if NSAT == 2:
                for c_ in all_cp[NS:]:
                    c_.start()
            wqvt_v[0:D // 2, :] = _pk(wqkv_v[:, 0:D].astype(F32).T)
            cp_moda.wait()
            cp_c.wait()
            if NSAT == 3:
                for c_ in all_cp[NS:]:
                    c_.start()
            modmm(0, 2)
            for q, r0 in enumerate(range(0, T, LR0)):
                ln1_chunk(0, 0, r0, xn0[q])
            cp_x1.wait()
            pr = [[proj_tasks((b, b, b), j) for j in range(NKB)] for b in range(3)]
            for fn, _, _ in ln1_tasks(1, 1):
                fn()
            for b in range(2):
                for j in range(NKB):
                    for fn, _, _ in pr[b][j][1]:
                        fn()
            cp_wk.wait()
            cp_wv.wait()
            cp_x2.wait()
            wqvt_v[D // 2:D, :] = _pk(wqkv_v[:, 2 * D:3 * D].astype(F32).T)
            for fn, c, _ in pr[0][0][0] + pr[0][0][2]:
                fn()
                acct(c)
            dense = []
            marks = []
            for b, j in ((0, 1), (1, 0), (1, 1)):
                dense += pr[b][j][0] + pr[b][j][2]
                marks.append(len(dense))
            groups = {}
            proj_groups(groups, (2, 2, 2))

            def waits():
                cp_x3.wait()
                cp_modb.wait()
                cp_wo.wait()

            groups['W'] = [(waits, 0, 0)]
            groups['m'] = mod_tasks(2, 6)
            groups['a'] = wo_tasks((0, 0, 0), 0, NG * 8)
            groups['b'] = wo_tasks((0, 0, 0), 1, 2 * NG * 8)
            n0 = len(dense)
            rest, ends = build(ORD0, groups)
            n = len(rest)
            rest = sprinkle(rest, [(ln1_tasks(3, 3), ends['W'] + L0R[0] * (n - ends['W']), ends['W'] + L0R[1] * (n - ends['W'])),
                                   (ln2_tasks(0, 0), ends['a'], ends['a'] + L0R[2] * (n - ends['a'])),
                                   (ln2_tasks(0, 1), ends['b'], ends['b'] + L0R[2] * (n - ends['b']))])
            l2 = ln1_tasks(2, 2)
            dense = sprinkle(dense, [(l2, 0, n0)]) + rest
            marks = [mk + sum(1 for q in range(len(l2)) if n0 * (q + 0.5) / len(l2) <= mk) for mk in marks]
            u0 = mk_units((0, 0, 0), [(False, False), (False, True)])
            u1 = mk_units((1, 1, 1), full)
            uneed = [0] * 32 + [marks[0]] * 32 + [marks[1]] * 32 + [marks[2]] * 32
            schedule(u0 + u1, dense, P0, uneed=uneed, barrier=waits)
            cp_w1.wait()
            cp_w2.wait()
            cp_xr.wait()
        elif gen:
            groups = {'a': wo_tasks((i, 0, 1), 0), 'b': wo_tasks((i, 0, 1), 1)}
            ffn_groups(groups, 0)
            proj_groups(groups, (0, 1, 2))
            dense, ends = build(ORD, groups)
            n = len(dense)
            dense = sprinkle(dense, [(ln1_tasks(jnp.minimum(i + 3, NBLK - 1), 1), L1R[0] * n, L1R[1] * n),
                                     (ln2_tasks(1, 0), ends['a'], L2R[0] * n), (ln2_tasks(1, 1), ends['b'], L2R[0] * n)])
            schedule(mk_units((0, 1, 1), full), dense, PG)
        elif kind == 'noproj':
            lb = NBLK - 1
            groups = {'a': wo_tasks((lb - 1,) * 3, 0), 'b': wo_tasks((lb - 1,) * 3, 1)}
            ffn_groups(groups, lb - 2)
            dense, ends = build(ORDN, groups)
            n = len(dense)
            dense = sprinkle(dense, [(ln2_tasks(lb - 1, 0), ends['a'], L2N[0] * n),
                                     (ln2_tasks(lb - 1, 1), ends['b'], L2N[0] * n)])
            gated = []
            for j in range(NKB):
                need = (j + 1) * NG * 8
                gated += wo_tasks((lb,) * 3, j, need) + ln2_tasks(lb, j, need)
            schedule(mk_units((lb,) * 3, full), dense, PN, gated)
        else:
            groups = {}
            ffn_groups(groups, i - 1)
            schedule([], build('ABCD', groups)[0], PG)

    variants = [
        (jnp.logical_and(i > 0, i < NBLK - 2), 'gen'),
        (i == 0, 'first'),
        (i == NBLK - 2, 'noproj'),
        (i > NBLK - 2, 'last'),
    ]
    for cond, kind in variants:
        pl.when(cond)(functools.partial(step, kind))


@jax.jit
def pallas_adaLN_cond__sliding_block__dense_activation_relu__prompt_kernel(A_x, A_wqkv, A_wo, B_x, B_w1, B_w2, c, w_mod):
    any_spec = pl.BlockSpec(memory_space=pl.ANY)
    return pl.pallas_call(
        _kernel,
        grid=(NBLK + 1,),
        in_specs=[
            any_spec, any_spec, any_spec, any_spec, any_spec, any_spec, any_spec,
        ],
        out_specs=pl.BlockSpec((None, T, D), lambda i: (0, jnp.maximum(i - 1, 0), 0)),
        out_shape=jax.ShapeDtypeStruct((1, S, D), BF16),
        scratch_shapes=[
            pltpu.VMEM((S, D), BF16),
            pltpu.VMEM((D, 6 * D), BF16),
            pltpu.VMEM((D, 3 * D), BF16),
            pltpu.VMEM((D, D), BF16),
            pltpu.VMEM((D, DFF), BF16),
            pltpu.VMEM((DFF, D), BF16),
            pltpu.VMEM((D, D), I32),
            pltpu.VMEM((8, 6 * D), F32),
            pltpu.VMEM((NBLK, D // 2, T), I32),
            pltpu.VMEM((H, S // 2, 128), I32),
            pltpu.VMEM((S // QB, D // 2, QB), I32),
            pltpu.VMEM((NBLK, T, D), BF16),
            pltpu.VMEM((NBLK + 1, 4, T, 128), BF16),
            pltpu.VMEM((NBLK, T, D), F32),
            pltpu.VMEM((NBLK, 4, T, 128), BF16),
            pltpu.VMEM((1, D), BF16),
            pltpu.SemaphoreType.DMA((14,)),
        ],
        compiler_params=pltpu.CompilerParams(
            dimension_semantics=("arbitrary",), vmem_limit_bytes=100 * 1024 * 1024),
    )(c, A_x, w_mod, A_wqkv, A_wo, B_w1, B_w2)
```

```python
import functools
import jax
import jax.numpy as jnp
from jax import lax
import jax.experimental.pallas as pl
import jax.experimental.pallas.tpu as pltpu

S = 2048
D = 512
H = 32
DH = 16
DFF = 1792
T = 256
QB = 128
HB = QB // 2
NG = 4
NBLK = S // T
NKB = T // QB
LOG2E = 1.4426950408889634
QSCALE = 0.25 * LOG2E
NEG = -1e30
EPS = 1e-5
PG = [0.95, 10.0, 40.0, 7.0, 0.0]
P0 = [0.93, 0.0, 28.0, 10.0, 1.0]
PN = [0.5, 10.0, 36.0, 8.0, 0.0]
ORD = 'acdebfghABCD'
ORD0 = 'dehWmcfabg'
L0R = [0.0, 0.8, 0.8]
ORDN = 'aAbCDZPQRXEGYH'
L1R = [0.1, 0.9]
L2R = [1.0]
QW = 3
KCH = 64
L2N = [0.7]
CMN = 16
HALF = 2
TRC = 128
CMAX = 64
NS = 3
DORD = '2103456789abc'
LR0 = 128
NSAT = 2
LR = 32
TIE = 1
F1R = 256
F2R = 128
NT = (((1,), (1,)), ((), ()))
F32 = jnp.float32
BF16 = jnp.bfloat16
I32 = jnp.int32


def _ln(xf, tie=None):
    mu = jnp.mean(xf, axis=-1, keepdims=True)
    if tie is not None:
        mu = jnp.where(tie[0], tie[1], mu)
    xc = xf - mu
    var = jnp.mean(xc * xc, axis=-1, keepdims=True)
    return xc * lax.rsqrt(var + EPS)


def _pk(v):
    return pltpu.bitcast(v.astype(BF16), I32)


def _up(v):
    return pltpu.bitcast(v, BF16)


def _dot(a, b):
    return jnp.dot(a, b, preferred_element_type=F32)


def _dot_nt(a, b):
    return lax.dot_general(a, b, NT, preferred_element_type=F32)


def _kernel(c_hbm, x_hbm, wmod_hbm, wqkv_hbm, wo_hbm, w1_hbm, w2_hbm, o_hbm,
            x_v, wmod_v, wqkv_v, wo_v, w1_v, w2_v, wqvt_v, mod_v, qt_v, k8_v, vt_v, ao_v, h_v, x1_v, h2_v,
            c_ref, o_v, sems, osems):
    i = pl.program_id(0)

    def cp(src, dst, k):
        return pltpu.make_async_copy(src, dst, sems.at[k])

    cp_moda = cp(wmod_hbm.at[:, 0:2 * D], wmod_v.at[:, 0:2 * D], 0)
    cp_x0 = cp(x_hbm.at[0, 0:T, :], x_v.at[0:T, :], 1)
    cp_wq = cp(wqkv_hbm.at[:, 0:D], wqkv_v.at[:, 0:D], 2)
    cp_x1 = cp(x_hbm.at[0, T:2 * T, :], x_v.at[T:2 * T, :], 3)
    cp_wk = cp(wqkv_hbm.at[:, D:2 * D], wqkv_v.at[:, D:2 * D], 4)
    cp_wv = cp(wqkv_hbm.at[:, 2 * D:3 * D], wqkv_v.at[:, 2 * D:3 * D], 5)
    cp_x2 = cp(x_hbm.at[0, 2 * T:3 * T, :], x_v.at[2 * T:3 * T, :], 6)
    cp_x3 = cp(x_hbm.at[0, 3 * T:4 * T, :], x_v.at[3 * T:4 * T, :], 7)
    cp_modb = cp(wmod_hbm.at[:, 2 * D:6 * D], wmod_v.at[:, 2 * D:6 * D], 8)
    cp_wo = cp(wo_hbm, wo_v, 9)
    cp_w1 = cp(w1_hbm, w1_v, 10)
    cp_w2 = cp(w2_hbm, w2_v, 11)
    cp_xr = cp(x_hbm.at[0, 4 * T:S, :], x_v.at[4 * T:S, :], 12)
    cp_c = cp(c_hbm, c_ref, 13)
    cps = [cp_moda, cp_x0, cp_wq, cp_x1, cp_wk, cp_wv, cp_x2, cp_x3, cp_modb, cp_wo, cp_w1, cp_w2, cp_xr]
    all_cp = [cps[int(ch, 16)] for ch in DORD]

    def cp_out(b, r0, n, k):
        start = b * T + r0
        if not isinstance(b, int):
            start = pl.multiple_of(start, n)
        return pltpu.make_async_copy(o_v.at[b, r0:r0 + n, :], o_hbm.at[0, pl.ds(start, n), :], osems.at[k])

    def silu_c():
        c = c_ref[...].astype(F32)
        sc = c * jax.nn.sigmoid(c)
        return jnp.broadcast_to(sc, (8, D)).astype(BF16)

    def modmm(lo, hi):
        mod_v[:, lo * D:hi * D] = _dot(silu_c(), wmod_v[:, lo * D:hi * D])

    def xrows(blk, r0, n, c0=0, c1=D):
        start = blk * T + r0
        if not isinstance(start, int):
            start = pl.multiple_of(start, n)
        return x_v[pl.ds(start, n), c0:c1]

    def step(kind):
        step_(kind)

    def step_(kind):
        first = kind == 'first'
        gen = kind == 'gen'
        if gen:
            qt_r = qt_v.at[pl.ds(i + 1, 2)]
            k8_r = k8_v.at[:, pl.ds(pl.multiple_of(i * (T // 2), T // 2), 3 * (T // 2)), :]
            vt_r = vt_v.at[pl.ds(i * NKB, 3 * NKB)]
            ao_r = ao_v.at[pl.ds(i, 2)]
            h_r = h_v.at[pl.ds(i + 2, 2)]
            x1_r = x1_v.at[pl.ds(i - 1, 2)]
            h2_r = h2_v.at[pl.ds(i - 1, 2)]
            o_r = o_v.at[pl.ds(i - 1, 1)]
        else:
            qt_r, k8_r, vt_r, ao_r, h_r, x1_r, h2_r, o_r = qt_v, k8_v, vt_v, ao_v, h_v, x1_v, h2_v, o_v

        loads = [0, 0, 0, 0]
        run = [0, 0, 0, 0]

        def acct(n):
            m = min(range(4), key=lambda k: (loads[k], k))
            loads[m] += max(n, 2)
            run[m] = run[m] + 1 if n <= 2 else 0

        lane = lax.broadcasted_iota(I32, (KCH, 128), 1)
        low_of = {w: ((lane // w) % 2) == 0 for w in (64, 32, 16)}
        bb = lax.broadcasted_iota(I32, (QB, QB), 0)
        aa = lax.broadcasted_iota(I32, (QB, QB), 1)
        tri = bb > aa
        diag = (lax.broadcasted_iota(I32, (HB, 128), 0) // 8) == (lax.broadcasted_iota(I32, (HB, 128), 1) // DH)
        use_l = (lax.broadcasted_iota(I32, (HB - 8, 128), 1) // DH) > (lax.broadcasted_iota(I32, (HB - 8, 128), 0) // 8)

        st = {}

        def acc(key, val):
            st[key] = val if key not in st else val + st[key]
            if val.shape[0] >= QB:
                st['last'] = st[key]
            return st[key]

        def tie(rows):
            v = st.get('last')
            if v is None or not TIE:
                return None
            return (i < 0, v[0:rows, 0:1])

        def ln1_chunk(xblk, hidx, r0, xn=None):
            if xn is None:
                xn = _ln(xrows(xblk, r0, LR).astype(F32), tie(LR))
            h = (xn * (1.0 + mod_v[0:1, D:2 * D]) + mod_v[0:1, 0:D]).astype(BF16)
            for k in range(4):
                h_r[hidx, k, r0:r0 + xn.shape[0], :] = h[:, k * 128:(k + 1) * 128]

        def ln2_chunk(widx, r0):
            xn = _ln(x1_r[widx, r0:r0 + LR, :], tie(LR))
            h = (xn * (1.0 + mod_v[0:1, 4 * D:5 * D]) + mod_v[0:1, 3 * D:4 * D]).astype(BF16)
            for k in range(4):
                h2_r[widx, k, r0:r0 + LR, :] = h[:, k * 128:(k + 1) * 128]

        def ln1_tasks(xblk, hidx, j=None):
            rows = range(0, T, LR) if j is None else range(j * QB, (j + 1) * QB, LR)
            return [(functools.partial(ln1_chunk, xblk, hidx, r0), 0, 0) for r0 in rows]

        def ln2_tasks(widx, j, need=0):
            return [(functools.partial(ln2_chunk, widx, r0), 0, need) for r0 in range(j * QB, (j + 1) * QB, LR)]

        def k_tile(blk, j, g, k):
            r = acc(('k', blk, j, g), _dot(h_r[blk[0], k, j * QB:(j + 1) * QB, :],
                                           wqkv_v[k * 128:(k + 1) * 128, D + g * 128:D + (g + 1) * 128]))
            if k == 3:
                kb = _pk(r)
                for r0 in range(0, HB, KCH):
                    vs = [kb[r0:r0 + KCH]]
                    for w in (64, 32, 16):
                        nxt = []
                        for v in vs:
                            rv = pltpu.roll(v, w, 1)
                            nxt += [jnp.where(low_of[w], v, rv), jnp.where(low_of[w], rv, v)]
                        vs = nxt
                    for hh in range(8):
                        k8_r[g * 8 + hh, pl.ds(blk[2] * (T // 2) + j * HB + r0, KCH), :] = vs[hh]

        def q_tile(blk, j, r, k):
            w = _up(wqvt_v[r * 128:(r + 1) * 128, k * 128:(k + 1) * 128])
            res = acc(('q', blk, r, j), _dot_nt(w, h_r[blk[0], k, j * QB:(j + 1) * QB, :]))
            if k == 3:
                qt_r[blk[1], r * 128:(r + 1) * 128, j * QB:(j + 1) * QB] = _pk(res * QSCALE)

        def v_tile(blk, j, r, k):
            w = _up(wqvt_v[D // 2 + r * 128:D // 2 + (r + 1) * 128, k * 128:(k + 1) * 128])
            res = acc(('v', blk, r, j), _dot_nt(w, h_r[blk[0], k, j * QB:(j + 1) * QB, :]))
            if k == 3:
                vt_r[blk[2] * NKB + j, r * 128:(r + 1) * 128, :] = _pk(res)

        def proj_tasks(blk, j):
            kt = [(functools.partial(k_tile, blk, j, g, k), 8, 0) for g in range(NG) for k in range(4)]
            qt = [(functools.partial(q_tile, blk, j, r, k), 16, 0) for r in range(2) for k in range(4)]
            vt = [(functools.partial(v_tile, blk, j, r, k), 16, 0) for r in range(2) for k in range(4)]
            return kt, qt, vt

        def wo_tile(blk, j, n, k):
            y = acc(('y', blk[1], j, n), _dot(ao_r[blk[1], j * QB:(j + 1) * QB, k * 128:(k + 1) * 128],
                                              wo_v[k * 128:(k + 1) * 128, n * 128:(n + 1) * 128]))
            if k == 3:
                ga = mod_v[0:1, 2 * D + n * 128:2 * D + (n + 1) * 128]
                x1_r[blk[2], j * QB:(j + 1) * QB, n * 128:(n + 1) * 128] = (
                    xrows(blk[0], j * QB, QB, n * 128, (n + 1) * 128).astype(F32) + ga * y)

        def wo_tasks(blk, j, need=0):
            return [(functools.partial(wo_tile, blk, j, n, k), 8, need) for n in range(4) for k in range(4)]

        def f1_tile(widx, r, c, k):
            f = acc(('f1', widx, r, c), _dot(h2_r[widx, k, r * F1R:(r + 1) * F1R, :],
                                       w1_v[k * 128:(k + 1) * 128, c * 128:(c + 1) * 128]))
            if k == 3:
                f = jnp.maximum(f, 0.0).astype(BF16)
                if F1R == T:
                    st['f', widx, 0, c] = f[0:QB]
                    st['f', widx, 1, c] = f[QB:]
                else:
                    st['f', widx, r, c] = f

        def f2_tile(widx, n, r, c):
            if F2R == T:
                f = jnp.concatenate([st['f', widx, 0, c], st['f', widx, 1, c]], axis=0)
            else:
                f = st['f', widx, r, c]
            z = acc(('z', widx, n, r), _dot(f, w2_v[c * 128:(c + 1) * 128, n * 128:(n + 1) * 128]))
            if c == DFF // 128 - 1:
                gb = mod_v[0:1, 5 * D + n * 128:5 * D + (n + 1) * 128]
                x1 = x1_r[widx, r * F2R:(r + 1) * F2R, n * 128:(n + 1) * 128]
                o_r[widx, r * F2R:(r + 1) * F2R, n * 128:(n + 1) * 128] = (x1 + gb * z).astype(BF16)

        def f1_tasks(widx, r):
            return [(functools.partial(f1_tile, widx, r, c, k), F1R // 16, 0)
                    for c in range(DFF // 128) for k in range(4)]

        def f2_tasks(widx, r):
            return [(functools.partial(f2_tile, widx, n, r, c), F2R // 16, 0)
                    for n in range(4) for c in range(DFF // 128)]

        def ffn_groups(groups, widx):
            groups['A'] = f1_tasks(widx, 0)
            groups['B'] = f1_tasks(widx, 1) if F1R != T else []
            groups['C'] = f2_tasks(widx, 0)
            groups['D'] = f2_tasks(widx, 1) if F2R != T else []

        def lhs(ib, head, j, has_first, has_mid):
            kl = (ib[1] * NKB + j) * HB
            if has_first:
                parts = [k8_r[head, pl.ds(kl, 8), :],
                         jnp.where(use_l, k8_r[head, pl.ds(kl + 8, HB - 8), :], k8_r[head, pl.ds(kl - 2 * HB, HB - 8), :]),
                         k8_r[head, pl.ds(kl - HB - 8, 8), :]]
            else:
                parts = [k8_r[head, pl.ds(kl, HB), :]]
            if has_mid:
                parts.append(k8_r[head, pl.ds(kl - HB, HB), :])
            return _up(jnp.concatenate(parts, axis=0) if len(parts) > 1 else parts[0])

        def qk_rows(has_first, has_mid):
            return (9 if has_first else 8) + (8 if has_mid else 0)

        def stage_a(g, hh, j, has_first, has_mid, ib):
            kwin = lhs(ib, g * 8 + hh, j, has_first, has_mid)
            r0 = g * 64 + hh * 8
            qh = qt_r[ib[0], r0:r0 + 8, j * QB:(j + 1) * QB]
            w = _up(jnp.where(diag, jnp.concatenate([qh] * 8, axis=0), 0))
            s_t = _dot(kwin, w)
            if has_first:
                sm = jnp.where(tri, s_t[DH:QB + DH], s_t[0:QB])
                rest = s_t[QB + DH:]
            else:
                sm = jnp.where(tri, NEG, s_t[0:QB])
                rest = s_t[QB:]
            if HALF and has_mid:
                st['s', g, hh, j] = (sm, jnp.max(sm, axis=0, keepdims=True), rest, jnp.max(rest, axis=0, keepdims=True))
                return
            s = jnp.concatenate([sm, rest], axis=0) if has_mid else sm
            m = jnp.max(s, axis=0, keepdims=True)
            st['s', g, hh, j] = (s, m)

        def pv_tiles(g, hh, j, has_first, has_mid, ib):
            qb = ib[1] * NKB + j
            r0 = g * 64 + hh * 8
            key = ('p', g, hh, j)

            half = HALF and has_mid

            def prep():
                if half:
                    s1, m1, s2, m2 = st.pop(('s', g, hh, j))
                    p1 = jnp.exp2(s1 - m1)
                    p2 = jnp.exp2(s2 - m2)
                    m = jnp.maximum(m1, m2)
                    a1 = jnp.exp2(m1 - m)
                    a2 = jnp.exp2(m2 - m)
                    if HALF == 1:
                        l = a1 * jnp.sum(p1, axis=0, keepdims=True) + a2 * jnp.sum(p2, axis=0, keepdims=True)
                    else:
                        l8 = a1 * jnp.sum(p1.reshape(QB // 8, 8, QB), axis=0) + a2 * jnp.sum(p2.reshape(QB // 8, 8, QB), axis=0)
                        l = jnp.sum(l8, axis=0, keepdims=True)
                    st[key] = (p1, p2, l, a1, a2)
                    return
                s, m = st.pop(('s', g, hh, j))
                p = jnp.exp2(s - m)
                st[key] = (p[0:QB], p[QB:], jnp.sum(p, axis=0, keepdims=True), None, None)

            def tile(which, is_first, is_last):
                if is_first:
                    prep()
                pm, p2, l, a1, a2 = st[key]
                if which == 'L':
                    pp = jnp.where(tri, 0.0, pm) if has_first else pm
                    vv = vt_r[qb, r0:r0 + 8, :]
                elif which == 'M':
                    pp = p2
                    vv = vt_r[qb - 1, r0:r0 + 8, :]
                else:
                    pp = jnp.where(tri, pm, 0.0)
                    vv = vt_r[qb - 2, r0:r0 + 8, :]
                okey = ('o', ib[1], g, hh, j, half and which == 'M')
                ot = acc(okey, _dot(_up(vv), pp.astype(BF16)))
                if is_last:
                    if half:
                        inv = 1.0 / l
                        st['on', g, j, hh] = (st['o', ib[1], g, hh, j, False] * (a1 * inv)
                                              + st['o', ib[1], g, hh, j, True] * (a2 * inv))
                    else:
                        st['on', g, j, hh] = ot * (1.0 / l)
                    if hh == 7:
                        og = jnp.concatenate([st['on', g, j, q] for q in range(8)], axis=0)
                        ao_r[ib[2], j * QB:(j + 1) * QB, g * 128:(g + 1) * 128] = og.T.astype(BF16)

            kinds = ['L'] + (['M'] if has_mid else []) + (['F'] if has_first else [])
            return [functools.partial(tile, w, q == 0, q == len(kinds) - 1) for q, w in enumerate(kinds)]

        def schedule(units, dense, params, gated=(), uneed=None, barrier=None):
            frac, lead, lag, maxin, PACE = params
            gated = list(gated)
            n = len(units)
            ucost = [qk_rows(u[3], u[4]) + 1 + u[3] + u[4] for u in units]
            dtot = sum(max(c, 2) for _, c, _ in dense + gated if c)
            tot = (dtot + sum(qk_rows(u[3], u[4]) + 2 * (1 + u[3] + u[4]) for u in units)) / 4.0
            base = min(loads)
            rate = frac * tot / max(n, 1)
            reserve = (1.0 - frac) * 4.0 * tot
            drem = dtot
            credit = lead
            nq = 0
            npv = 0
            pvq = []
            qk_time = {}
            nd = 0
            while nq < n or npv < n or dense or gated:
                now = min(loads) - base
                m = min(range(4), key=lambda k: (loads[k], k))
                pv_ok = npv < nq and now >= qk_time[npv] + lag
                qk_can = nq < n and nq - npv < maxin and (uneed is None or nd >= uneed[nq])
                if PACE:
                    spacing = max(drem - reserve, 0.0) * ucost[nq] / sum(ucost[nq:]) if nq < n else 0.0
                    qk_due = qk_can and credit >= spacing
                else:
                    qk_due = qk_can and now >= nq * rate - lead
                quiet = any(t[0] is barrier for t in dense[:QW]) and dense[0][2] <= npv
                if gated and npv >= gated[0][2]:
                    choice = 'g'
                elif quiet:
                    choice = 'd'
                elif pv_ok and run[m] < 2:
                    choice = 'pv'
                elif qk_due:
                    choice = 'qk'
                elif dense and dense[0][2] <= npv:
                    choice = 'd'
                elif qk_can:
                    choice = 'qk'
                else:
                    choice = 'pv'
                if choice == 'pv':
                    if not pvq:
                        pvq = pv_tiles(*units[npv])
                    fn = pvq.pop(0)
                    fn()
                    acct(1)
                    if not pvq:
                        npv += 1
                elif choice == 'qk':
                    qk_time[nq] = now
                    if PACE:
                        credit = min(credit - spacing, CMAX if first else CMN)
                    stage_a(*units[nq])
                    acct(qk_rows(units[nq][3], units[nq][4]))
                    nq += 1
                else:
                    fn, c, _ = (dense if choice == 'd' else gated).pop(0)
                    nd += choice == 'd'
                    fn()
                    if c:
                        acct(c)
                        drem -= max(c, 2)
                        credit += max(c, 2)

        def mk_units(ib, flags):
            return [(g, hh, j) + flags[j] + (ib,) for j in range(NKB) for g in range(NG) for hh in range(8)]

        def mod_tasks(lo, hi):
            def t(q):
                mod_v[:, q * 128:(q + 1) * 128] = _dot(silu_c(), wmod_v[:, q * 128:(q + 1) * 128])
            return [(functools.partial(t, q), 8, 0) for q in range(lo * 4, hi * 4)]

        def build(order, groups):
            dense = []
            ends = {}
            for ch in order:
                dense = dense + groups[ch]
                ends[ch] = len(dense)
            return dense, ends

        def sprinkle(dense, extras):
            ins = []
            for tasks, lo, hi in extras:
                hi = max(hi, lo)
                for q, t in enumerate(tasks):
                    ins.append((lo + (hi - lo) * (q + 0.5) / len(tasks), t))
            ins.sort(key=lambda e: e[0])
            out = []
            for pos, t in enumerate(dense):
                while ins and ins[0][0] <= pos:
                    out.append(ins.pop(0)[1])
                out.append(t)
            return out + [e[1] for e in ins]

        def proj_groups(groups, blk):
            groups['c'], groups['d'], groups['e'] = proj_tasks(blk, 0)
            groups['f'], groups['g'], groups['h'] = proj_tasks(blk, 1)

        full = [(True, True)] * NKB
        if first:
            for c_ in all_cp[:NS]:
                c_.start()
            cp_c.start()
            cp_x0.wait()
            if NSAT == 1:
                for c_ in all_cp[NS:]:
                    c_.start()
            xn_v = x1_v.at[NBLK - 1]

            def stats(q, carry):
                rows = pl.ds(pl.multiple_of(q * LR0, LR0), LR0)
                xn_v[rows, :] = _ln(x_v[rows, :].astype(F32))
                return carry

            lax.fori_loop(0, T // LR0, stats, 0)
            cp_wq.wait()
            if NSAT == 2:
                for c_ in all_cp[NS:]:
                    c_.start()

            def tr(q, carry):
                cols = pl.ds(pl.multiple_of(q * TRC, TRC), TRC)
                wqvt_v[pl.ds(pl.multiple_of(q * (TRC // 2), TRC // 2), TRC // 2), :] = _pk(wqkv_v[:, cols].astype(F32).T)
                return carry

            lax.fori_loop(0, D // TRC, tr, 0)
            cp_moda.wait()
            cp_c.wait()
            if NSAT == 3:
                for c_ in all_cp[NS:]:
                    c_.start()
            modmm(0, 2)
            for q, r0 in enumerate(range(0, T, LR0)):
                ln1_chunk(0, 0, r0, xn_v[r0:r0 + LR0, :])
            cp_x1.wait()
            pr = [[proj_tasks((b, b, b), j) for j in range(NKB)] for b in range(3)]
            for fn, _, _ in ln1_tasks(1, 1):
                fn()
            for b in range(2):
                for j in range(NKB):
                    for fn, _, _ in pr[b][j][1]:
                        fn()
            cp_wk.wait()
            cp_wv.wait()
            cp_x2.wait()
            wqvt_v[D // 2:D, :] = _pk(wqkv_v[:, 2 * D:3 * D].astype(F32).T)
            for fn, c, _ in pr[0][0][0] + pr[0][0][2]:
                fn()
                acct(c)
            dense = []
            marks = []
            for b, j in ((0, 1), (1, 0), (1, 1)):
                dense += pr[b][j][0] + pr[b][j][2]
                marks.append(len(dense))
            groups = {}
            proj_groups(groups, (2, 2, 2))

            def waits():
                cp_x3.wait()
                cp_modb.wait()
                cp_wo.wait()

            groups['W'] = [(waits, 0, 0)]
            groups['m'] = mod_tasks(2, 6)
            groups['a'] = wo_tasks((0, 0, 0), 0, NG * 8)
            groups['b'] = wo_tasks((0, 0, 0), 1, 2 * NG * 8)
            n0 = len(dense)
            rest, ends = build(ORD0, groups)
            n = len(rest)
            rest = sprinkle(rest, [(ln1_tasks(3, 3), ends['W'] + L0R[0] * (n - ends['W']), ends['W'] + L0R[1] * (n - ends['W'])),
                                   (ln2_tasks(0, 0), ends['a'], ends['a'] + L0R[2] * (n - ends['a'])),
                                   (ln2_tasks(0, 1), ends['b'], ends['b'] + L0R[2] * (n - ends['b']))])
            l2 = ln1_tasks(2, 2)
            dense = sprinkle(dense, [(l2, 0, n0)]) + rest
            marks = [mk + sum(1 for q in range(len(l2)) if n0 * (q + 0.5) / len(l2) <= mk) for mk in marks]
            u0 = mk_units((0, 0, 0), [(False, False), (False, True)])
            u1 = mk_units((1, 1, 1), full)
            uneed = [0] * 32 + [marks[0]] * 32 + [marks[1]] * 32 + [marks[2]] * 32
            schedule(u0 + u1, dense, P0, uneed=uneed, barrier=waits)
            cp_w1.wait()
            cp_w2.wait()
            cp_xr.wait()
        elif gen:
            groups = {'a': wo_tasks((i, 0, 1), 0), 'b': wo_tasks((i, 0, 1), 1)}
            ffn_groups(groups, 0)
            proj_groups(groups, (0, 1, 2))
            dense, ends = build(ORD, groups)
            n = len(dense)
            dense = sprinkle(dense, [(ln1_tasks(jnp.minimum(i + 3, NBLK - 1), 1), L1R[0] * n, L1R[1] * n),
                                     (ln2_tasks(1, 0), ends['a'], L2R[0] * n), (ln2_tasks(1, 1), ends['b'], L2R[0] * n)])
            schedule(mk_units((0, 1, 1), full), dense, PG)
        else:
            last = NBLK - 1
            g5, g6, g7 = {}, {}, {}
            ffn_groups(g5, last - 2)
            ffn_groups(g6, last - 1)
            ffn_groups(g7, last)
            nt = DFF // 128
            hr = T // 2
            nu = NKB * NG * 8

            def cp_col(n):
                return pltpu.make_async_copy(o_v.at[last, hr:T, n * 128:(n + 1) * 128],
                                             o_hbm.at[0, last * T + hr:S, n * 128:(n + 1) * 128], osems.at[NBLK + n])

            tail = []
            for n in range(4):
                tail += g7['D'][n * nt:(n + 1) * nt]
                if n < 3:
                    tail.append((functools.partial(lambda n: cp_col(n).start(), n), 0, 0))
            groups = {'a': wo_tasks((last - 1,) * 3, 0), 'b': wo_tasks((last - 1,) * 3, 1),
                      'A': g5['A'], 'C': g5['C'], 'D': g5['D'],
                      'P': g6['A'], 'Q': g6['C'], 'R': g6['D'],
                      'E': [(fn, c, nu) for fn, c, _ in g7['A']], 'G': g7['C'], 'H': tail,
                      'Z': [(lambda: cp_out(last - 2, 0, T, last - 2).start(), 0, 0)],
                      'X': [(lambda: cp_out(last - 1, 0, T, last - 1).start(), 0, 0)],
                      'Y': [(lambda: cp_out(last, 0, hr, last).start(), 0, 0)]}
            for b in range(last - 3):
                cp_out(b, 0, T, b).wait()
            dense, ends = build(ORDN, groups)
            np_ = ends['P'] - len(groups['P'])
            dense = sprinkle(dense, [(ln2_tasks(last - 1, 0), ends['a'], ends['a'] + L2N[0] * (np_ - ends['a'])),
                                     (ln2_tasks(last - 1, 1), ends['b'], ends['b'] + L2N[0] * (np_ - ends['b']))])
            gated = []
            for j in range(NKB):
                need = (j + 1) * NG * 8
                gated += wo_tasks((last,) * 3, j, need) + ln2_tasks(last, j, need)
            schedule(mk_units((last,) * 3, full), dense, PN, gated)
            cp_col(3).start()
            for b in range(last - 3, last):
                cp_out(b, 0, T, b).wait()
            cp_out(last, 0, hr, last).wait()
            for n in range(4):
                cp_col(n).wait()

    variants = [
        (jnp.logical_and(i > 0, i < NBLK - 2), 'gen'),
        (i == 0, 'first'),
        (i == NBLK - 2, 'final'),
    ]
    for cond, kind in variants:
        pl.when(cond)(functools.partial(step, kind))

    @pl.when(jnp.logical_and(i > 0, i < NBLK - 2))
    def _():
        cp_out(i - 1, 0, T, i - 1).start()


@jax.jit
def pallas_adaLN_cond__sliding_block__dense_activation_relu__prompt_kernel(A_x, A_wqkv, A_wo, B_x, B_w1, B_w2, c, w_mod):
    any_spec = pl.BlockSpec(memory_space=pl.ANY)
    return pl.pallas_call(
        _kernel,
        grid=(NBLK - 1,),
        in_specs=[
            any_spec, any_spec, any_spec, any_spec, any_spec, any_spec, any_spec,
        ],
        out_specs=any_spec,
        out_shape=jax.ShapeDtypeStruct((1, S, D), BF16),
        scratch_shapes=[
            pltpu.VMEM((S, D), BF16),
            pltpu.VMEM((D, 6 * D), BF16),
            pltpu.VMEM((D, 3 * D), BF16),
            pltpu.VMEM((D, D), BF16),
            pltpu.VMEM((D, DFF), BF16),
            pltpu.VMEM((DFF, D), BF16),
            pltpu.VMEM((D, D), I32),
            pltpu.VMEM((8, 6 * D), F32),
            pltpu.VMEM((NBLK, D // 2, T), I32),
            pltpu.VMEM((H, S // 2, 128), I32),
            pltpu.VMEM((S // QB, D // 2, QB), I32),
            pltpu.VMEM((NBLK, T, D), BF16),
            pltpu.VMEM((NBLK + 1, 4, T, 128), BF16),
            pltpu.VMEM((NBLK, T, D), F32),
            pltpu.VMEM((NBLK, 4, T, 128), BF16),
            pltpu.VMEM((1, D), BF16),
            pltpu.VMEM((NBLK, T, D), BF16),
            pltpu.SemaphoreType.DMA((14,)),
            pltpu.SemaphoreType.DMA((NBLK + 4,)),
        ],
        compiler_params=pltpu.CompilerParams(
            dimension_semantics=("arbitrary",), vmem_limit_bytes=100 * 1024 * 1024),
    )(c, A_x, w_mod, A_wqkv, A_wo, B_w1, B_w2)
```

```python
import functools
import jax
import jax.numpy as jnp
from jax import lax
import jax.experimental.pallas as pl
import jax.experimental.pallas.tpu as pltpu

S = 2048
D = 512
H = 32
DH = 16
DFF = 1792
T = 256
QB = 128
HB = QB // 2
NG = 4
NBLK = S // T
NKB = T // QB
LOG2E = 1.4426950408889634
QSCALE = 0.25 * LOG2E
NEG = -1e30
EPS = 1e-5
PG = [0.9, 0.0, 32.0, 5.0, 0.0]
P0 = [0.93, 0.0, 28.0, 10.0, 1.0]
PN = [0.5, 10.0, 36.0, 8.0, 0.0]
ORD = 'acdebfghABCD'
ORD0 = 'dehWmcfabg'
L0R = [0.0, 0.8, 0.8]
ORDN = 'aAbCDZPQRXEGYH'
L1R = [0.2, 0.9]
L2R = [0.95]
QW = 3
KCH = 64
L2N = [0.7]
CMN = 16
HALF = 2
TRC = 128
CMAX = 64
NS = 3
DORD = '2103456789abc'
LR0 = 128
NSAT = 2
LRG = 16
LRF = 32
LRL = 32
TIE = 1
F1R = 256
F2R = 128
NT = (((1,), (1,)), ((), ()))
F32 = jnp.float32
BF16 = jnp.bfloat16
I32 = jnp.int32


def _ln(xf, tie=None):
    mu = jnp.mean(xf, axis=-1, keepdims=True)
    if tie is not None:
        mu = jnp.where(tie[0], tie[1], mu)
    xc = xf - mu
    var = jnp.mean(xc * xc, axis=-1, keepdims=True)
    return xc * lax.rsqrt(var + EPS)


def _pk(v):
    return pltpu.bitcast(v.astype(BF16), I32)


def _up(v):
    return pltpu.bitcast(v, BF16)


def _dot(a, b):
    return jnp.dot(a, b, preferred_element_type=F32)


def _dot_nt(a, b):
    return lax.dot_general(a, b, NT, preferred_element_type=F32)


def _kernel(c_hbm, x_hbm, wmod_hbm, wqkv_hbm, wo_hbm, w1_hbm, w2_hbm, o_hbm,
            x_v, wmod_v, wqkv_v, wo_v, w1_v, w2_v, wqvt_v, mod_v, qt_v, k8_v, vt_v, ao_v, h_v, x1_v, h2_v,
            c_ref, o_v, sems, osems):
    i = pl.program_id(0)

    def cp(src, dst, k):
        return pltpu.make_async_copy(src, dst, sems.at[k])

    cp_moda = cp(wmod_hbm.at[:, 0:2 * D], wmod_v.at[:, 0:2 * D], 0)
    cp_x0 = cp(x_hbm.at[0, 0:T, :], x_v.at[0:T, :], 1)
    cp_wq = cp(wqkv_hbm.at[:, 0:D], wqkv_v.at[:, 0:D], 2)
    cp_x1 = cp(x_hbm.at[0, T:2 * T, :], x_v.at[T:2 * T, :], 3)
    cp_wk = cp(wqkv_hbm.at[:, D:2 * D], wqkv_v.at[:, D:2 * D], 4)
    cp_wv = cp(wqkv_hbm.at[:, 2 * D:3 * D], wqkv_v.at[:, 2 * D:3 * D], 5)
    cp_x2 = cp(x_hbm.at[0, 2 * T:3 * T, :], x_v.at[2 * T:3 * T, :], 6)
    cp_x3 = cp(x_hbm.at[0, 3 * T:4 * T, :], x_v.at[3 * T:4 * T, :], 7)
    cp_modb = cp(wmod_hbm.at[:, 2 * D:6 * D], wmod_v.at[:, 2 * D:6 * D], 8)
    cp_wo = cp(wo_hbm, wo_v, 9)
    cp_w1 = cp(w1_hbm, w1_v, 10)
    cp_w2 = cp(w2_hbm, w2_v, 11)
    cp_xr = cp(x_hbm.at[0, 4 * T:S, :], x_v.at[4 * T:S, :], 12)
    cp_c = cp(c_hbm, c_ref, 13)
    cps = [cp_moda, cp_x0, cp_wq, cp_x1, cp_wk, cp_wv, cp_x2, cp_x3, cp_modb, cp_wo, cp_w1, cp_w2, cp_xr]
    all_cp = [cps[int(ch, 16)] for ch in DORD]

    def cp_out(b, r0, n, k):
        start = b * T + r0
        if not isinstance(b, int):
            start = pl.multiple_of(start, n)
        return pltpu.make_async_copy(o_v.at[b, r0:r0 + n, :], o_hbm.at[0, pl.ds(start, n), :], osems.at[k])

    def silu_c():
        c = c_ref[...].astype(F32)
        sc = c * jax.nn.sigmoid(c)
        return jnp.broadcast_to(sc, (8, D)).astype(BF16)

    def modmm(lo, hi):
        mod_v[:, lo * D:hi * D] = _dot(silu_c(), wmod_v[:, lo * D:hi * D])

    def xrows(blk, r0, n, c0=0, c1=D):
        start = blk * T + r0
        if not isinstance(start, int):
            start = pl.multiple_of(start, n)
        return x_v[pl.ds(start, n), c0:c1]

    def step(kind):
        step_(kind)

    def step_(kind):
        first = kind == 'first'
        gen = kind == 'gen'
        LR = LRG if gen else LRF if first else LRL
        if gen:
            qt_r = qt_v.at[pl.ds(i + 1, 2)]
            k8_r = k8_v.at[:, pl.ds(pl.multiple_of(i * (T // 2), T // 2), 3 * (T // 2)), :]
            vt_r = vt_v.at[pl.ds(i * NKB, 3 * NKB)]
            ao_r = ao_v.at[pl.ds(i, 2)]
            h_r = h_v.at[pl.ds(i + 2, 2)]
            x1_r = x1_v.at[pl.ds(i - 1, 2)]
            h2_r = h2_v.at[pl.ds(i - 1, 2)]
            o_r = o_v.at[pl.ds(i - 1, 1)]
        else:
            qt_r, k8_r, vt_r, ao_r, h_r, x1_r, h2_r, o_r = qt_v, k8_v, vt_v, ao_v, h_v, x1_v, h2_v, o_v

        loads = [0, 0, 0, 0]
        run = [0, 0, 0, 0]

        def acct(n):
            m = min(range(4), key=lambda k: (loads[k], k))
            loads[m] += max(n, 2)
            run[m] = run[m] + 1 if n <= 2 else 0

        lane = lax.broadcasted_iota(I32, (KCH, 128), 1)
        low_of = {w: ((lane // w) % 2) == 0 for w in (64, 32, 16)}
        bb = lax.broadcasted_iota(I32, (QB, QB), 0)
        aa = lax.broadcasted_iota(I32, (QB, QB), 1)
        tri = bb > aa
        diag = (lax.broadcasted_iota(I32, (HB, 128), 0) // 8) == (lax.broadcasted_iota(I32, (HB, 128), 1) // DH)
        use_l = (lax.broadcasted_iota(I32, (HB - 8, 128), 1) // DH) > (lax.broadcasted_iota(I32, (HB - 8, 128), 0) // 8)

        st = {}

        def acc(key, val):
            st[key] = val if key not in st else val + st[key]
            if val.shape[0] >= QB:
                st['last'] = st[key]
            return st[key]

        def tie(rows):
            v = st.get('last')
            if v is None or not TIE:
                return None
            return (i < 0, v[0:rows, 0:1])

        def ln1_chunk(xblk, hidx, r0, xn=None):
            if xn is None:
                xn = _ln(xrows(xblk, r0, LR).astype(F32), tie(LR))
            h = (xn * (1.0 + mod_v[0:1, D:2 * D]) + mod_v[0:1, 0:D]).astype(BF16)
            for k in range(4):
                h_r[hidx, k, r0:r0 + xn.shape[0], :] = h[:, k * 128:(k + 1) * 128]

        def ln2_chunk(widx, r0):
            xn = _ln(x1_r[widx, r0:r0 + LR, :], tie(LR))
            h = (xn * (1.0 + mod_v[0:1, 4 * D:5 * D]) + mod_v[0:1, 3 * D:4 * D]).astype(BF16)
            for k in range(4):
                h2_r[widx, k, r0:r0 + LR, :] = h[:, k * 128:(k + 1) * 128]

        def ln1_tasks(xblk, hidx, j=None):
            rows = range(0, T, LR) if j is None else range(j * QB, (j + 1) * QB, LR)
            return [(functools.partial(ln1_chunk, xblk, hidx, r0), 0, 0) for r0 in rows]

        def ln2_tasks(widx, j, need=0):
            return [(functools.partial(ln2_chunk, widx, r0), 0, need) for r0 in range(j * QB, (j + 1) * QB, LR)]

        def k_tile(blk, j, g, k):
            r = acc(('k', blk, j, g), _dot(h_r[blk[0], k, j * QB:(j + 1) * QB, :],
                                           wqkv_v[k * 128:(k + 1) * 128, D + g * 128:D + (g + 1) * 128]))
            if k == 3:
                kb = _pk(r)
                for r0 in range(0, HB, KCH):
                    vs = [kb[r0:r0 + KCH]]
                    for w in (64, 32, 16):
                        nxt = []
                        for v in vs:
                            rv = pltpu.roll(v, w, 1)
                            nxt += [jnp.where(low_of[w], v, rv), jnp.where(low_of[w], rv, v)]
                        vs = nxt
                    for hh in range(8):
                        k8_r[g * 8 + hh, pl.ds(blk[2] * (T // 2) + j * HB + r0, KCH), :] = vs[hh]

        def q_tile(blk, j, r, k):
            w = _up(wqvt_v[r * 128:(r + 1) * 128, k * 128:(k + 1) * 128])
            res = acc(('q', blk, r, j), _dot_nt(w, h_r[blk[0], k, j * QB:(j + 1) * QB, :]))
            if k == 3:
                qt_r[blk[1], r * 128:(r + 1) * 128, j * QB:(j + 1) * QB] = _pk(res * QSCALE)

        def v_tile(blk, j, r, k):
            w = _up(wqvt_v[D // 2 + r * 128:D // 2 + (r + 1) * 128, k * 128:(k + 1) * 128])
            res = acc(('v', blk, r, j), _dot_nt(w, h_r[blk[0], k, j * QB:(j + 1) * QB, :]))
            if k == 3:
                vt_r[blk[2] * NKB + j, r * 128:(r + 1) * 128, :] = _pk(res)

        def proj_tasks(blk, j):
            kt = [(functools.partial(k_tile, blk, j, g, k), 8, 0) for g in range(NG) for k in range(4)]
            qt = [(functools.partial(q_tile, blk, j, r, k), 16, 0) for r in range(2) for k in range(4)]
            vt = [(functools.partial(v_tile, blk, j, r, k), 16, 0) for r in range(2) for k in range(4)]
            return kt, qt, vt

        def wo_tile(blk, j, n, k):
            y = acc(('y', blk[1], j, n), _dot(ao_r[blk[1], j * QB:(j + 1) * QB, k * 128:(k + 1) * 128],
                                              wo_v[k * 128:(k + 1) * 128, n * 128:(n + 1) * 128]))
            if k == 3:
                ga = mod_v[0:1, 2 * D + n * 128:2 * D + (n + 1) * 128]
                x1_r[blk[2], j * QB:(j + 1) * QB, n * 128:(n + 1) * 128] = (
                    xrows(blk[0], j * QB, QB, n * 128, (n + 1) * 128).astype(F32) + ga * y)

        def wo_tasks(blk, j, need=0):
            return [(functools.partial(wo_tile, blk, j, n, k), 8, need) for n in range(4) for k in range(4)]

        def f1_tile(widx, r, c, k):
            f = acc(('f1', widx, r, c), _dot(h2_r[widx, k, r * F1R:(r + 1) * F1R, :],
                                       w1_v[k * 128:(k + 1) * 128, c * 128:(c + 1) * 128]))
            if k == 3:
                f = jnp.maximum(f, 0.0).astype(BF16)
                if F1R == T:
                    st['f', widx, 0, c] = f[0:QB]
                    st['f', widx, 1, c] = f[QB:]
                else:
                    st['f', widx, r, c] = f

        def f2_tile(widx, n, r, c):
            if F2R == T:
                f = jnp.concatenate([st['f', widx, 0, c], st['f', widx, 1, c]], axis=0)
            else:
                f = st['f', widx, r, c]
            z = acc(('z', widx, n, r), _dot(f, w2_v[c * 128:(c + 1) * 128, n * 128:(n + 1) * 128]))
            if c == DFF // 128 - 1:
                gb = mod_v[0:1, 5 * D + n * 128:5 * D + (n + 1) * 128]
                x1 = x1_r[widx, r * F2R:(r + 1) * F2R, n * 128:(n + 1) * 128]
                o_r[widx, r * F2R:(r + 1) * F2R, n * 128:(n + 1) * 128] = (x1 + gb * z).astype(BF16)

        def f1_tasks(widx, r):
            return [(functools.partial(f1_tile, widx, r, c, k), F1R // 16, 0)
                    for c in range(DFF // 128) for k in range(4)]

        def f2_tasks(widx, r):
            return [(functools.partial(f2_tile, widx, n, r, c), F2R // 16, 0)
                    for n in range(4) for c in range(DFF // 128)]

        def ffn_groups(groups, widx):
            groups['A'] = f1_tasks(widx, 0)
            groups['B'] = f1_tasks(widx, 1) if F1R != T else []
            groups['C'] = f2_tasks(widx, 0)
            groups['D'] = f2_tasks(widx, 1) if F2R != T else []

        def lhs(ib, head, j, has_first, has_mid):
            kl = (ib[1] * NKB + j) * HB
            if has_first:
                parts = [k8_r[head, pl.ds(kl, 8), :],
                         jnp.where(use_l, k8_r[head, pl.ds(kl + 8, HB - 8), :], k8_r[head, pl.ds(kl - 2 * HB, HB - 8), :]),
                         k8_r[head, pl.ds(kl - HB - 8, 8), :]]
            else:
                parts = [k8_r[head, pl.ds(kl, HB), :]]
            if has_mid:
                parts.append(k8_r[head, pl.ds(kl - HB, HB), :])
            return _up(jnp.concatenate(parts, axis=0) if len(parts) > 1 else parts[0])

        def qk_rows(has_first, has_mid):
            return (9 if has_first else 8) + (8 if has_mid else 0)

        def stage_a(g, hh, j, has_first, has_mid, ib):
            kwin = lhs(ib, g * 8 + hh, j, has_first, has_mid)
            r0 = g * 64 + hh * 8
            qh = qt_r[ib[0], r0:r0 + 8, j * QB:(j + 1) * QB]
            w = _up(jnp.where(diag, jnp.concatenate([qh] * 8, axis=0), 0))
            s_t = _dot(kwin, w)
            if has_first:
                sm = jnp.where(tri, s_t[DH:QB + DH], s_t[0:QB])
                rest = s_t[QB + DH:]
            else:
                sm = jnp.where(tri, NEG, s_t[0:QB])
                rest = s_t[QB:]
            if HALF and has_mid:
                st['s', g, hh, j] = (sm, jnp.max(sm, axis=0, keepdims=True), rest, jnp.max(rest, axis=0, keepdims=True))
                return
            s = jnp.concatenate([sm, rest], axis=0) if has_mid else sm
            m = jnp.max(s, axis=0, keepdims=True)
            st['s', g, hh, j] = (s, m)

        def pv_tiles(g, hh, j, has_first, has_mid, ib):
            qb = ib[1] * NKB + j
            r0 = g * 64 + hh * 8
            key = ('p', g, hh, j)

            half = HALF and has_mid

            def prep():
                if half:
                    s1, m1, s2, m2 = st.pop(('s', g, hh, j))
                    p1 = jnp.exp2(s1 - m1)
                    p2 = jnp.exp2(s2 - m2)
                    m = jnp.maximum(m1, m2)
                    a1 = jnp.exp2(m1 - m)
                    a2 = jnp.exp2(m2 - m)
                    if HALF == 1:
                        l = a1 * jnp.sum(p1, axis=0, keepdims=True) + a2 * jnp.sum(p2, axis=0, keepdims=True)
                    else:
                        l8 = a1 * jnp.sum(p1.reshape(QB // 8, 8, QB), axis=0) + a2 * jnp.sum(p2.reshape(QB // 8, 8, QB), axis=0)
                        l = jnp.sum(l8, axis=0, keepdims=True)
                    st[key] = (p1, p2, l, a1, a2)
                    return
                s, m = st.pop(('s', g, hh, j))
                p = jnp.exp2(s - m)
                st[key] = (p[0:QB], p[QB:], jnp.sum(p, axis=0, keepdims=True), None, None)

            def tile(which, is_first, is_last):
                if is_first:
                    prep()
                pm, p2, l, a1, a2 = st[key]
                if which == 'L':
                    pp = jnp.where(tri, 0.0, pm) if has_first else pm
                    vv = vt_r[qb, r0:r0 + 8, :]
                elif which == 'M':
                    pp = p2
                    vv = vt_r[qb - 1, r0:r0 + 8, :]
                else:
                    pp = jnp.where(tri, pm, 0.0)
                    vv = vt_r[qb - 2, r0:r0 + 8, :]
                okey = ('o', ib[1], g, hh, j, half and which == 'M')
                ot = acc(okey, _dot(_up(vv), pp.astype(BF16)))
                if is_last:
                    if half:
                        inv = 1.0 / l
                        st['on', g, j, hh] = (st['o', ib[1], g, hh, j, False] * (a1 * inv)
                                              + st['o', ib[1], g, hh, j, True] * (a2 * inv))
                    else:
                        st['on', g, j, hh] = ot * (1.0 / l)
                    if hh == 7:
                        og = jnp.concatenate([st['on', g, j, q] for q in range(8)], axis=0)
                        ao_r[ib[2], j * QB:(j + 1) * QB, g * 128:(g + 1) * 128] = og.T.astype(BF16)

            kinds = ['L'] + (['M'] if has_mid else []) + (['F'] if has_first else [])
            return [functools.partial(tile, w, q == 0, q == len(kinds) - 1) for q, w in enumerate(kinds)]

        def schedule(units, dense, params, gated=(), uneed=None, barrier=None):
            frac, lead, lag, maxin, PACE = params
            gated = list(gated)
            n = len(units)
            ucost = [qk_rows(u[3], u[4]) + 1 + u[3] + u[4] for u in units]
            dtot = sum(max(c, 2) for _, c, _ in dense + gated if c)
            tot = (dtot + sum(qk_rows(u[3], u[4]) + 2 * (1 + u[3] + u[4]) for u in units)) / 4.0
            base = min(loads)
            rate = frac * tot / max(n, 1)
            reserve = (1.0 - frac) * 4.0 * tot
            drem = dtot
            credit = lead
            nq = 0
            npv = 0
            pvq = []
            qk_time = {}
            nd = 0
            while nq < n or npv < n or dense or gated:
                now = min(loads) - base
                m = min(range(4), key=lambda k: (loads[k], k))
                pv_ok = npv < nq and now >= qk_time[npv] + lag
                qk_can = nq < n and nq - npv < maxin and (uneed is None or nd >= uneed[nq])
                if PACE:
                    spacing = max(drem - reserve, 0.0) * ucost[nq] / sum(ucost[nq:]) if nq < n else 0.0
                    qk_due = qk_can and credit >= spacing
                else:
                    qk_due = qk_can and now >= nq * rate - lead
                quiet = any(t[0] is barrier for t in dense[:QW]) and dense[0][2] <= npv
                if gated and npv >= gated[0][2]:
                    choice = 'g'
                elif quiet:
                    choice = 'd'
                elif pv_ok and run[m] < 2:
                    choice = 'pv'
                elif qk_due:
                    choice = 'qk'
                elif dense and dense[0][2] <= npv:
                    choice = 'd'
                elif qk_can:
                    choice = 'qk'
                else:
                    choice = 'pv'
                if choice == 'pv':
                    if not pvq:
                        pvq = pv_tiles(*units[npv])
                    fn = pvq.pop(0)
                    fn()
                    acct(1)
                    if not pvq:
                        npv += 1
                elif choice == 'qk':
                    qk_time[nq] = now
                    if PACE:
                        credit = min(credit - spacing, CMAX if first else CMN)
                    stage_a(*units[nq])
                    acct(qk_rows(units[nq][3], units[nq][4]))
                    nq += 1
                else:
                    fn, c, _ = (dense if choice == 'd' else gated).pop(0)
                    nd += choice == 'd'
                    fn()
                    if c:
                        acct(c)
                        drem -= max(c, 2)
                        credit += max(c, 2)

        def mk_units(ib, flags):
            return [(g, hh, j) + flags[j] + (ib,) for j in range(NKB) for g in range(NG) for hh in range(8)]

        def mod_tasks(lo, hi):
            def t(q):
                mod_v[:, q * 128:(q + 1) * 128] = _dot(silu_c(), wmod_v[:, q * 128:(q + 1) * 128])
            return [(functools.partial(t, q), 8, 0) for q in range(lo * 4, hi * 4)]

        def build(order, groups):
            dense = []
            ends = {}
            for ch in order:
                dense = dense + groups[ch]
                ends[ch] = len(dense)
            return dense, ends

        def sprinkle(dense, extras):
            ins = []
            for tasks, lo, hi in extras:
                hi = max(hi, lo)
                for q, t in enumerate(tasks):
                    ins.append((lo + (hi - lo) * (q + 0.5) / len(tasks), t))
            ins.sort(key=lambda e: e[0])
            out = []
            for pos, t in enumerate(dense):
                while ins and ins[0][0] <= pos:
                    out.append(ins.pop(0)[1])
                out.append(t)
            return out + [e[1] for e in ins]

        def proj_groups(groups, blk):
            groups['c'], groups['d'], groups['e'] = proj_tasks(blk, 0)
            groups['f'], groups['g'], groups['h'] = proj_tasks(blk, 1)

        full = [(True, True)] * NKB
        if first:
            for c_ in all_cp[:NS]:
                c_.start()
            cp_c.start()
            cp_x0.wait()
            if NSAT == 1:
                for c_ in all_cp[NS:]:
                    c_.start()
            xn_v = x1_v.at[NBLK - 1]

            def stats(q, carry):
                rows = pl.ds(pl.multiple_of(q * LR0, LR0), LR0)
                xn_v[rows, :] = _ln(x_v[rows, :].astype(F32))
                return carry

            lax.fori_loop(0, T // LR0, stats, 0)
            cp_wq.wait()
            if NSAT == 2:
                for c_ in all_cp[NS:]:
                    c_.start()

            def tr(q, carry):
                cols = pl.ds(pl.multiple_of(q * TRC, TRC), TRC)
                wqvt_v[pl.ds(pl.multiple_of(q * (TRC // 2), TRC // 2), TRC // 2), :] = _pk(wqkv_v[:, cols].astype(F32).T)
                return carry

            lax.fori_loop(0, D // TRC, tr, 0)
            cp_moda.wait()
            cp_c.wait()
            if NSAT == 3:
                for c_ in all_cp[NS:]:
                    c_.start()
            modmm(0, 2)
            for q, r0 in enumerate(range(0, T, LR0)):
                ln1_chunk(0, 0, r0, xn_v[r0:r0 + LR0, :])
            cp_x1.wait()
            pr = [[proj_tasks((b, b, b), j) for j in range(NKB)] for b in range(3)]
            for fn, _, _ in ln1_tasks(1, 1):
                fn()
            for b in range(2):
                for j in range(NKB):
                    for fn, _, _ in pr[b][j][1]:
                        fn()
            cp_wk.wait()
            cp_wv.wait()
            cp_x2.wait()
            wqvt_v[D // 2:D, :] = _pk(wqkv_v[:, 2 * D:3 * D].astype(F32).T)
            for fn, c, _ in pr[0][0][0] + pr[0][0][2]:
                fn()
                acct(c)
            dense = []
            marks = []
            for b, j in ((0, 1), (1, 0), (1, 1)):
                dense += pr[b][j][0] + pr[b][j][2]
                marks.append(len(dense))
            groups = {}
            proj_groups(groups, (2, 2, 2))

            def waits():
                cp_x3.wait()
                cp_modb.wait()
                cp_wo.wait()

            groups['W'] = [(waits, 0, 0)]
            groups['m'] = mod_tasks(2, 6)
            groups['a'] = wo_tasks((0, 0, 0), 0, NG * 8)
            groups['b'] = wo_tasks((0, 0, 0), 1, 2 * NG * 8)
            n0 = len(dense)
            rest, ends = build(ORD0, groups)
            n = len(rest)
            rest = sprinkle(rest, [(ln1_tasks(3, 3), ends['W'] + L0R[0] * (n - ends['W']), ends['W'] + L0R[1] * (n - ends['W'])),
                                   (ln2_tasks(0, 0), ends['a'], ends['a'] + L0R[2] * (n - ends['a'])),
                                   (ln2_tasks(0, 1), ends['b'], ends['b'] + L0R[2] * (n - ends['b']))])
            l2 = ln1_tasks(2, 2)
            dense = sprinkle(dense, [(l2, 0, n0)]) + rest
            marks = [mk + sum(1 for q in range(len(l2)) if n0 * (q + 0.5) / len(l2) <= mk) for mk in marks]
            u0 = mk_units((0, 0, 0), [(False, False), (False, True)])
            u1 = mk_units((1, 1, 1), full)
            uneed = [0] * 32 + [marks[0]] * 32 + [marks[1]] * 32 + [marks[2]] * 32
            schedule(u0 + u1, dense, P0, uneed=uneed, barrier=waits)
            cp_w1.wait()
            cp_w2.wait()
            cp_xr.wait()
        elif gen:
            groups = {'a': wo_tasks((i, 0, 1), 0), 'b': wo_tasks((i, 0, 1), 1)}
            ffn_groups(groups, 0)
            proj_groups(groups, (0, 1, 2))
            dense, ends = build(ORD, groups)
            n = len(dense)
            dense = sprinkle(dense, [(ln1_tasks(jnp.minimum(i + 3, NBLK - 1), 1), L1R[0] * n, L1R[1] * n),
                                     (ln2_tasks(1, 0), ends['a'], L2R[0] * n), (ln2_tasks(1, 1), ends['b'], L2R[0] * n)])
            schedule(mk_units((0, 1, 1), full), dense, PG)
        else:
            last = NBLK - 1
            g5, g6, g7 = {}, {}, {}
            ffn_groups(g5, last - 2)
            ffn_groups(g6, last - 1)
            ffn_groups(g7, last)
            nt = DFF // 128
            hr = T // 2
            nu = NKB * NG * 8

            def cp_col(n):
                return pltpu.make_async_copy(o_v.at[last, hr:T, n * 128:(n + 1) * 128],
                                             o_hbm.at[0, last * T + hr:S, n * 128:(n + 1) * 128], osems.at[NBLK + n])

            tail = []
            for n in range(4):
                tail += g7['D'][n * nt:(n + 1) * nt]
                if n < 3:
                    tail.append((functools.partial(lambda n: cp_col(n).start(), n), 0, 0))
            groups = {'a': wo_tasks((last - 1,) * 3, 0), 'b': wo_tasks((last - 1,) * 3, 1),
                      'A': g5['A'], 'C': g5['C'], 'D': g5['D'],
                      'P': g6['A'], 'Q': g6['C'], 'R': g6['D'],
                      'E': [(fn, c, nu) for fn, c, _ in g7['A']], 'G': g7['C'], 'H': tail,
                      'Z': [(lambda: cp_out(last - 2, 0, T, last - 2).start(), 0, 0)],
                      'X': [(lambda: cp_out(last - 1, 0, T, last - 1).start(), 0, 0)],
                      'Y': [(lambda: cp_out(last, 0, hr, last).start(), 0, 0)]}
            for b in range(last - 3):
                cp_out(b, 0, T, b).wait()
            dense, ends = build(ORDN, groups)
            np_ = ends['P'] - len(groups['P'])
            dense = sprinkle(dense, [(ln2_tasks(last - 1, 0), ends['a'], ends['a'] + L2N[0] * (np_ - ends['a'])),
                                     (ln2_tasks(last - 1, 1), ends['b'], ends['b'] + L2N[0] * (np_ - ends['b']))])
            gated = []
            for j in range(NKB):
                need = (j + 1) * NG * 8
                gated += wo_tasks((last,) * 3, j, need) + ln2_tasks(last, j, need)
            schedule(mk_units((last,) * 3, full), dense, PN, gated)
            cp_col(3).start()
            for b in range(last - 3, last):
                cp_out(b, 0, T, b).wait()
            cp_out(last, 0, hr, last).wait()
            for n in range(4):
                cp_col(n).wait()

    variants = [
        (jnp.logical_and(i > 0, i < NBLK - 2), 'gen'),
        (i == 0, 'first'),
        (i == NBLK - 2, 'final'),
    ]
    for cond, kind in variants:
        pl.when(cond)(functools.partial(step, kind))

    @pl.when(jnp.logical_and(i > 0, i < NBLK - 2))
    def _():
        cp_out(i - 1, 0, T, i - 1).start()


@jax.jit
def pallas_adaLN_cond__sliding_block__dense_activation_relu__prompt_kernel(A_x, A_wqkv, A_wo, B_x, B_w1, B_w2, c, w_mod):
    any_spec = pl.BlockSpec(memory_space=pl.ANY)
    return pl.pallas_call(
        _kernel,
        grid=(NBLK - 1,),
        in_specs=[
            any_spec, any_spec, any_spec, any_spec, any_spec, any_spec, any_spec,
        ],
        out_specs=any_spec,
        out_shape=jax.ShapeDtypeStruct((1, S, D), BF16),
        scratch_shapes=[
            pltpu.VMEM((S, D), BF16),
            pltpu.VMEM((D, 6 * D), BF16),
            pltpu.VMEM((D, 3 * D), BF16),
            pltpu.VMEM((D, D), BF16),
            pltpu.VMEM((D, DFF), BF16),
            pltpu.VMEM((DFF, D), BF16),
            pltpu.VMEM((D, D), I32),
            pltpu.VMEM((8, 6 * D), F32),
            pltpu.VMEM((NBLK, D // 2, T), I32),
            pltpu.VMEM((H, S // 2, 128), I32),
            pltpu.VMEM((S // QB, D // 2, QB), I32),
            pltpu.VMEM((NBLK, T, D), BF16),
            pltpu.VMEM((NBLK + 1, 4, T, 128), BF16),
            pltpu.VMEM((NBLK, T, D), F32),
            pltpu.VMEM((NBLK, 4, T, 128), BF16),
            pltpu.VMEM((1, D), BF16),
            pltpu.VMEM((NBLK, T, D), BF16),
            pltpu.SemaphoreType.DMA((14,)),
            pltpu.SemaphoreType.DMA((NBLK + 4,)),
        ],
        compiler_params=pltpu.CompilerParams(
            dimension_semantics=("arbitrary",), vmem_limit_bytes=100 * 1024 * 1024),
    )(c, A_x, w_mod, A_wqkv, A_wo, B_w1, B_w2)
```
